```python
import os as _os
_os.environ.setdefault('JAX_PLATFORMS', 'cpu')
import jax
import jax.numpy as jnp

def _softmax(x, axis=-1):
    return jax.nn.softmax(x, axis=axis)

def _gelu(x):
    return jax.nn.gelu(x, approximate=True)

def _silu(x):
    return jax.nn.silu(x)

def _sigmoid(x):
    return jax.nn.sigmoid(x)

def _layernorm(x, axis=-1, eps=1e-05):
    m = jnp.mean(x, axis=axis, keepdims=True)
    v = jnp.var(x, axis=axis, keepdims=True)
    return (x - m) / jnp.sqrt(v + eps)

def _scatter_add(tgt, idx, src, axis=0):
    return tgt.at[idx].add(src)

def _segment_sum(src, seg, n):
    return jax.ops.segment_sum(src, seg, n)

class _Rng:

    def __init__(self, key):
        self._k = key

    def _next(self):
        self._k, sub = jax.random.split(self._k)
        return sub

    def normal(self, shape):
        return jax.random.normal(self._next(), shape, dtype=jnp.bfloat16)

    def randint(self, lo, hi, shape):
        return jax.random.randint(self._next(), shape, lo, hi, dtype=jnp.int32)

    def uniform(self, shape, lo=0.0, hi=1.0):
        return jax.random.uniform(self._next(), shape, jnp.bfloat16, lo, hi)

    def permutation(self, n):
        return jax.random.permutation(self._next(), n)
kernel_name = 'adaLN_cond__mha_block__geglu_ffn__prompt'

def setup_inputs():
    _rng = _Rng(jax.random.key(int.from_bytes(__import__("os").urandom(4), "little")))
    _w = lambda a: (lambda t: t.astype(jnp.bfloat16) if jnp.issubdtype(t.dtype, jnp.floating) else t)(jnp.asarray(a))

    def _A_setup():
        B, S, D, H = (1, 2048, 640, 32)
        return {'x': _w((lambda *s: _rng.normal(s) * 0.05)(B, S, D)), 'wqkv': _w((lambda *s: _rng.normal(s) * 0.05)(D, 3 * D)), 'wo': _w((lambda *s: _rng.normal(s) * 0.05)(D, D))}
    _A_in = _A_setup()

    def _B_setup():
        B, S, D, F = (1, 2048, 640, 1728)
        return {'x': _w((lambda *s: _rng.normal(s) * 0.05)(B, S, D)), 'w_gate': _w((lambda *s: _rng.normal(s) * 0.05)(D, F)), 'w_up': _w((lambda *s: _rng.normal(s) * 0.05)(D, F)), 'w_down': _w((lambda *s: _rng.normal(s) * 0.05)(F, D))}
    _B_in = _B_setup()
    return {'A_x': _A_in['x'], 'A_wqkv': _A_in['wqkv'], 'A_wo': _A_in['wo'], 'B_x': _B_in['x'], 'B_w_gate': _B_in['w_gate'], 'B_w_up': _B_in['w_up'], 'B_w_down': _B_in['w_down'], 'c': _w((lambda *s: _rng.normal(s) * 0.05)(1, 640) * 8.0), 'w_mod': _w((lambda *s: _rng.normal(s) * 0.05)(640, 6 * 640) * 640 ** (-0.5) * 8.0)}

def reference(A_x, A_wqkv, A_wo, B_x, B_w_gate, B_w_up, B_w_down, c, w_mod):

    def _A_ref(x, wqkv, wo):
        B, S, D = x.shape
        H = 32
        Dh = D // H
        qkv = (lambda x, *d: x.transpose(*d))((x @ wqkv).reshape(B, S, 3, H, Dh), 2, 0, 3, 1, 4)
        q, k, v = (qkv[0], qkv[1], qkv[2])
        scores = jnp.einsum('bhqd,bhkd->bhqk', q, k) * Dh ** (-0.5)
        p = _softmax(scores, axis=-1)
        o = jnp.einsum('bhqk,bhkd->bhqd', p, v)
        return (lambda x, *d: x.transpose(*d))(o, 0, 2, 1, 3).reshape(B, S, D) @ wo

    def _B_ref(x, w_gate, w_up, w_down):
        return _gelu(x @ w_gate) * (x @ w_up) @ w_down
    x = A_x
    mod = (_silu(c) @ w_mod).reshape(c.shape[0], 6, 1, -1)
    sa, ca, ga, sb, cb, gb = (mod[:, 0].copy(), mod[:, 1].copy(), mod[:, 2].copy(), mod[:, 3].copy(), mod[:, 4].copy(), mod[:, 5].copy())
    h = _layernorm(x, axis=-1) * (1 + ca) + sa
    x = x + ga * _A_ref(h, A_wqkv, A_wo)
    h = _layernorm(x, axis=-1) * (1 + cb) + sb
    x = x + gb * _B_ref(h, B_w_gate, B_w_up, B_w_down)
    return x
```

```python
import functools
import math

import jax
import jax.numpy as jnp
import jax.experimental.pallas as pl
import jax.experimental.pallas.tpu as pltpu

S = 2048
D = 640
H = 32
DH = 20
F = 1728
LANES = 128
NG = 6
TQ = 512
NQ = S // TQ
TK = 256
NK = S // TK
VR = 32
R1 = 256
R3 = 256
FC = 384
EPS = 1e-5
QSCALE = (DH ** -0.5) * math.log2(math.e)
STRADDLE = [h for h in range(H) if (DH * h) % LANES > LANES - DH]

_NT = (((1,), (1,)), ((), ()))


def _layernorm(xf):
    m = jnp.mean(xf, axis=-1, keepdims=True)
    xc = xf - m
    v = jnp.mean(xc * xc, axis=-1, keepdims=True)
    return xc * jax.lax.rsqrt(v + EPS)


def _kernel(x_ref, wqkv_ref, wo_ref, wg_ref, wu_ref, wd_ref, c_ref, wmod_ref,
            out_ref,
            mod_ref, wx_ref, wvt_ref, k_ref, q_ref, vt_ref, ot_ref,
            sa_ref, sb_ref, ma_ref, mb_ref, oc_ref):
    f32 = jnp.float32
    bf16 = jnp.bfloat16

    c = c_ref[...].astype(f32)
    sc = (c * jax.nn.sigmoid(c)).astype(bf16)
    sc = jnp.broadcast_to(sc, (16, D))
    mod_ref[...] = jnp.dot(sc, wmod_ref[...], preferred_element_type=f32)

    lane = jax.lax.broadcasted_iota(jnp.int32, (D, LANES), 1)
    for part, base in ((0, D), (1, 0)):
        acc = jnp.zeros((D, LANES), f32)
        for j, h in enumerate(STRADDLE):
            lo = base + DH * h
            t0 = (lo // LANES) * LANES
            win = wqkv_ref[:, t0:t0 + 2 * LANES].astype(f32)
            sh = (DH * j - (lo - t0)) % (2 * LANES)
            rolled = pltpu.roll(win, sh, 1)[:, :LANES]
            acc = jnp.where((lane >= DH * j) & (lane < DH * (j + 1)), rolled, acc)
        wx_ref[:, part * LANES:(part + 1) * LANES] = acc.astype(bf16)
    wvt_ref[...] = wqkv_ref[:, 2 * D:3 * D].T

    sa = mod_ref[0:1, 0 * D:1 * D]
    ca1 = 1.0 + mod_ref[0:1, 1 * D:2 * D]
    row32 = jax.lax.broadcasted_iota(jnp.int32, (VR, R1), 0)

    def proj_body(i, carry):
        r0 = pl.multiple_of(i * R1, R1)
        xf = x_ref[pl.ds(r0, R1), :].astype(f32)
        h = (_layernorm(xf) * ca1 + sa).astype(bf16)
        qk = jnp.dot(h, wqkv_ref[:, 0:2 * D], preferred_element_type=f32)
        ex = jnp.dot(h, wx_ref[...], preferred_element_type=f32)
        for g in range(5):
            q_ref[g, pl.ds(r0, R1), :] = (qk[:, g * LANES:(g + 1) * LANES] * QSCALE).astype(bf16)
            k_ref[g, pl.ds(r0, R1), :] = qk[:, D + g * LANES:D + (g + 1) * LANES].astype(bf16)
        k_ref[5, pl.ds(r0, R1), :] = ex[:, 0:LANES].astype(bf16)
        q_ref[5, pl.ds(r0, R1), :] = (ex[:, LANES:2 * LANES] * QSCALE).astype(bf16)
        vt = jax.lax.dot_general(wvt_ref[...], h, _NT, preferred_element_type=f32)
        oc_ref[0:D, 0:R1] = vt
        oc_ref[D:D + 16, 0:R1] = jnp.zeros((16, R1), f32)
        for hd in range(H):
            a0 = (DH * hd // 8) * 8
            off = DH * hd - a0
            win = oc_ref[a0:a0 + VR + 8, 0:R1]
            win = win[off:off + VR]
            win = jnp.where(row32 < DH, win, jnp.where(row32 == DH, 1.0, 0.0))
            vt_ref[hd, i] = win.astype(bf16)
        return carry

    jax.lax.fori_loop(0, S // R1, proj_body, 0)

    lane_q = jax.lax.broadcasted_iota(jnp.int32, (TQ, LANES), 1)

    def head_info(b):
        hd = b // NQ
        qt = b % NQ
        lo = hd * DH
        g = lo // LANES
        o = lo % LANES
        st = o > LANES - DH
        g2 = jnp.where(st, 5, g)
        o2 = jnp.where(st, g * DH, o)
        return hd, qt, g2, o2

    def load_q(b):
        hd, qt, g, o = head_info(b)
        q = q_ref[g, pl.ds(pl.multiple_of(qt * TQ, TQ), TQ), :].astype(f32)
        q = jnp.where((lane_q >= o) & (lane_q < o + DH), q, 0.0).astype(bf16)
        return q, g

    def qk_chunk(q, g, c, s_ref, m8):
        s = jax.lax.dot_general(k_ref[g, c * TK:(c + 1) * TK, :], q, _NT,
                                preferred_element_type=f32)
        s_ref[c * TK:(c + 1) * TK, :] = s
        cm = jnp.max(s.reshape(TK // 8, 8, TQ), axis=0)
        return cm if m8 is None else jnp.maximum(m8, cm)

    def pv_chunk(hd, c, s_ref, m, acc):
        p = jnp.exp2(s_ref[c * TK:(c + 1) * TK, :] - m).astype(bf16)
        o = jnp.dot(vt_ref[hd, c], p, preferred_element_type=f32)
        return o if acc is None else acc + o

    def pv_finish(b, acc):
        hd, qt, _, _ = head_info(b)
        ot_ref[hd, qt] = acc * (1.0 / acc[DH:DH + 1, :])

    def step(b_qk, s_w, m_w, b_pv, s_r, m_r):
        q, g = load_q(b_qk)
        hd = b_pv // NQ
        m = m_r[...]
        m8 = None
        acc = None
        for c in range(NK):
            m8 = qk_chunk(q, g, c, s_w, m8)
            acc = pv_chunk(hd, c, s_r, m, acc)
        m_w[...] = jnp.max(m8, axis=0, keepdims=True)
        pv_finish(b_pv, acc)

    q0, g0 = load_q(0)
    m8 = None
    for c in range(NK):
        m8 = qk_chunk(q0, g0, c, sa_ref, m8)
    ma_ref[...] = jnp.max(m8, axis=0, keepdims=True)

    NB = H * NQ

    def attn_body(j, carry):
        b = 2 * j
        step(b + 1, sb_ref, mb_ref, b, sa_ref, ma_ref)
        step(jnp.minimum(b + 2, NB - 1), sa_ref, ma_ref, b + 1, sb_ref, mb_ref)
        return carry

    jax.lax.fori_loop(0, NB // 2, attn_body, 0)

    ga = mod_ref[0:1, 2 * D:3 * D]
    sb = mod_ref[0:1, 3 * D:4 * D]
    cb1 = 1.0 + mod_ref[0:1, 4 * D:5 * D]
    gb = mod_ref[0:1, 5 * D:6 * D]
    per = TQ // R3

    def ffn_body(i, carry):
        r0 = pl.multiple_of(i * R3, R3)
        qt = i // per
        sub = i % per
        for hd in range(H):
            if per == 1:
                blk = ot_ref[hd, qt]
            else:
                full = ot_ref[hd, qt]
                blk = full[:, 0:R3]
                for t in range(1, per):
                    blk = jnp.where(sub == t, full[:, t * R3:(t + 1) * R3], blk)
            oc_ref[DH * hd:DH * hd + DH, 0:R3] = blk[0:DH]
        o = oc_ref[0:D, 0:R3].astype(bf16).T
        attn = jnp.dot(o, wo_ref[...], preferred_element_type=f32)
        x1 = x_ref[pl.ds(r0, R3), :].astype(f32) + ga * attn
        h2 = (_layernorm(x1) * cb1 + sb).astype(bf16)
        y = None
        f0 = 0
        while f0 < F:
            fc = min(FC, F - f0)
            g = jnp.dot(h2, wg_ref[:, f0:f0 + fc], preferred_element_type=f32)
            u = jnp.dot(h2, wu_ref[:, f0:f0 + fc], preferred_element_type=f32)
            a = (jax.nn.gelu(g, approximate=True) * u).astype(bf16)
            d = jnp.dot(a, wd_ref[f0:f0 + fc, :], preferred_element_type=f32)
            y = d if y is None else y + d
            f0 += fc
        out_ref[pl.ds(r0, R3), :] = (x1 + gb * y).astype(out_ref.dtype)
        return carry

    jax.lax.fori_loop(0, S // R3, ffn_body, 0)


@jax.jit
def pallas_adaLN_cond__mha_block__geglu_ffn__prompt_kernel(
    A_x: jax.Array,
    A_wqkv: jax.Array,
    A_wo: jax.Array,
    B_x: jax.Array,
    B_w_gate: jax.Array,
    B_w_up: jax.Array,
    B_w_down: jax.Array,
    c: jax.Array,
    w_mod: jax.Array,
):
    del B_x
    f32 = jnp.float32
    bf16 = jnp.bfloat16
    x2 = A_x.reshape(S, D)
    RC = max(R1, R3)
    out = pl.pallas_call(
        _kernel,
        out_shape=jax.ShapeDtypeStruct((S, D), A_x.dtype),
        scratch_shapes=[
            pltpu.VMEM((16, 6 * D), f32),
            pltpu.VMEM((D, 2 * LANES), bf16),
            pltpu.VMEM((D, D), bf16),
            pltpu.VMEM((NG, S, LANES), bf16),
            pltpu.VMEM((NG, S, LANES), bf16),
            pltpu.VMEM((H, S // R1, VR, R1), bf16),
            pltpu.VMEM((H, NQ, VR, TQ), f32),
            pltpu.VMEM((S, TQ), f32),
            pltpu.VMEM((S, TQ), f32),
            pltpu.VMEM((1, TQ), f32),
            pltpu.VMEM((1, TQ), f32),
            pltpu.VMEM((D + 16, RC), f32),
        ],
        compiler_params=pltpu.CompilerParams(vmem_limit_bytes=110 * 1024 * 1024),
        name="adaln_block",
    )(x2, A_wqkv, A_wo, B_w_gate, B_w_up, B_w_down, c, w_mod)
    return out.reshape(A_x.shape)
```

```python
import math
import os

import jax
import jax.numpy as jnp
import jax.experimental.pallas as pl
import jax.experimental.pallas.tpu as pltpu
import contextlib


def _scope(name):
    return jax.named_scope(name) if os.environ.get("K_SCOPES") else contextlib.nullcontext()

S = 2048
D = 640
H = 32
DH = 20
F = 1728
LANES = 128
NG = 6
TQ = 512
NQ = S // TQ
TC = LANES
NC = S // TC
HALF = NC // 2
NB = H * NQ
NSTEP = int(os.environ.get("K_NSTEP", 4))
SKEW = int(os.environ.get("K_SKEW", 1))
VR = 32
R1 = 256
NX = S // R1
R3 = 256
N3 = S // R3
FCS = tuple(int(v) for v in os.environ.get("K_FCS", "384,640,640").split(","))
MIDPOS = int(os.environ.get("K_MID", 1))
LATEPOS = int(os.environ.get("K_LATE", 2))
EPS = 1e-5
QSCALE = (DH ** -0.5) * math.log2(math.e)
STRADDLE = [h for h in range(H) if (DH * h) % LANES > LANES - DH]
FMAIN = (F // LANES) * LANES
FREM = F - FMAIN
MDL = int(os.environ.get("K_MDL", 2))
QVU = int(os.environ.get("K_QVU", 2))
XEARLY = 2

_NT = (((1,), (1,)), ((), ()))

(_S_C, _S_MODA, _S_MODA2, _S_WQ, _S_WK, _S_WV, _S_MODB, _S_WO, _S_WG, _S_WU, _S_WD, _S_OUT, _S_XA,
 _S_XB) = range(14)


def _layernorm(xf):
    m = jnp.mean(xf, axis=-1, keepdims=True)
    xc = xf - m
    v = jnp.mean(xc * xc, axis=-1, keepdims=True)
    return xc * jax.lax.rsqrt(v + EPS)


def _kernel(x_hbm, wqkv_hbm, wo_hbm, wgt_hbm, wut_hbm, wd_hbm, c_hbm, wmod_hbm,
            out_hbm,
            x_ref, wqkv_ref, wo_ref, wgt_ref, wut_ref, wd_ref, c_ref, wmod_ref, ostage_ref,
            mod_ref, wt_ref, h_ref, qx_ref, ov_ref, wgul_ref,
            k_ref, qt_ref, vt_ref, ot_ref,
            sa_ref, sa2_ref, sb_ref, sb2_ref, ma_ref, mb_ref, m8_ref, oc_ref,
            hh_ref, x1_ref, oo_ref,
            zero_ref, sems):
    f32 = jnp.float32
    bf16 = jnp.bfloat16

    def cp(src, dst, slot):
        return pltpu.make_async_copy(src, dst, sems.at[slot])

    XE = XEARLY * R1
    c_cp = cp(c_hbm, c_ref, _S_C)
    moda_cp = cp(wmod_hbm.at[:, 0:2 * D], wmod_ref.at[:, 0:2 * D], _S_MODA)
    modb_cp = cp(wmod_hbm.at[:, 2 * D:6 * D], wmod_ref.at[:, 2 * D:6 * D], _S_MODB)
    wq_cp = cp(wqkv_hbm.at[:, 0:D], wqkv_ref.at[:, 0:D], _S_WQ)
    wk_cp = cp(wqkv_hbm.at[:, D:2 * D], wqkv_ref.at[:, D:2 * D], _S_WK)
    wv_cp = cp(wqkv_hbm.at[:, 2 * D:3 * D], wqkv_ref.at[:, 2 * D:3 * D], _S_WV)
    wo_cp = cp(wo_hbm, wo_ref, _S_WO)
    wg_cp = cp(wgt_hbm, wgt_ref, _S_WG)
    wu_cp = cp(wut_hbm, wut_ref, _S_WU)
    wd_cp = cp(wd_hbm, wd_ref, _S_WD)
    xa_cp = cp(x_hbm.at[0:XE, :], x_ref.at[0:XE, :], _S_XA)
    xb_cp = cp(x_hbm.at[XE:S, :], x_ref.at[XE:S, :], _S_XB)

    zero_ref[0] = 0
    c_cp.start()
    xa_cp.start()
    moda_cp.start()
    wk_cp.start()

    c_cp.wait()
    c = c_ref[...].astype(f32)
    sc = jnp.broadcast_to((c * jax.nn.sigmoid(c)).astype(bf16), (16, D))
    oc_ref[D:D + 16, :] = jnp.zeros((16, oc_ref.shape[1]), f32)
    with _scope("w_xa"):
        xa_cp.wait()
    xn0 = _layernorm(x_ref[0:R1, :].astype(f32))
    with _scope("w_moda"):
        moda_cp.wait()
    xb_cp.start()
    wq_cp.start()
    wv_cp.start()
    mod_ref[:, 0:2 * D] = jnp.dot(sc, wmod_ref[:, 0:2 * D], preferred_element_type=f32)
    sa = mod_ref[0:1, 0 * D:1 * D]
    ca1 = 1.0 + mod_ref[0:1, 1 * D:2 * D]

    def ln1(i):
        xf = x_ref[i * R1:(i + 1) * R1, :].astype(f32)
        h_ref[i] = (_layernorm(xf) * ca1 + sa).astype(bf16)

    lane_k = jax.lax.broadcasted_iota(jnp.int32, (R1, LANES), 1)

    def kproj(i):
        h = h_ref[i]
        kk = jnp.dot(h, wqkv_ref[:, D:2 * D], preferred_element_type=f32)
        for g in range(5):
            k_ref[g, i * R1:(i + 1) * R1, :] = kk[:, g * LANES:(g + 1) * LANES].astype(bf16)
        kx = jnp.zeros((R1, LANES), f32)
        for j, hd in enumerate(STRADDLE):
            lo = DH * hd
            t = lo // LANES
            sh = (DH * j - lo) % LANES
            a = pltpu.roll(kk[:, t * LANES:(t + 1) * LANES], sh, 1)
            b = pltpu.roll(kk[:, (t + 1) * LANES:(t + 2) * LANES], sh, 1)
            n_a = (t + 1) * LANES - lo
            kx = jnp.where((lane_k >= DH * j) & (lane_k < DH * j + n_a), a,
                           jnp.where((lane_k >= DH * j + n_a) & (lane_k < DH * (j + 1)), b, kx))
        k_ref[5, i * R1:(i + 1) * R1, :] = kx.astype(bf16)

    h_ref[0] = (xn0 * ca1 + sa).astype(bf16)
    with _scope("w_wk"):
        wk_cp.wait()
    for i in range(NX):
        if i + 1 == XEARLY:
            xb_cp.wait()
            modb_cp.start()
            wo_cp.start()
            wg_cp.start()
            wu_cp.start()
            wd_cp.start()
        if i == XEARLY:
            wq_cp.wait()
            wv_cp.wait()
            wt_ref[0:D, :] = wqkv_ref[:, 0:D].T
            wt_ref[D:2 * D, :] = wqkv_ref[:, 2 * D:3 * D].T
        if i + 1 < NX:
            ln1(i + 1)
        kproj(i)

    row32 = jax.lax.broadcasted_iota(jnp.int32, (VR, R1), 0)

    def qvproj(i):
        h = h_ref[i]
        qv = jax.lax.dot_general(wt_ref[...], h, _NT, preferred_element_type=f32)
        oc_ref[0:D, :] = qv[0:D] * QSCALE
        for g in range(5):
            qt_ref[g, i] = oc_ref[g * LANES:(g + 1) * LANES, :].astype(bf16)
        for j, hd in enumerate(STRADDLE):
            qx_ref[DH * j:DH * (j + 1), :] = oc_ref[DH * hd:DH * (hd + 1), :]
        qt_ref[5, i] = qx_ref[...].astype(bf16)
        ov_ref[0:D, :] = qv[D:2 * D]
        for hd in range(H):
            a0 = (DH * hd // 8) * 8
            off = DH * hd - a0
            win = ov_ref[a0:a0 + VR + 8, :]
            win = win[off:off + VR]
            win = jnp.where(row32 < DH, win, jnp.where(row32 == DH, 1.0, 0.0))
            vt_ref[hd, i] = win.astype(bf16)

    qx_ref[...] = jnp.zeros(qx_ref.shape, f32)
    ov_ref[D:D + 16, :] = jnp.zeros((16, R1), f32)

    def qv_body(j, carry):
        for t in range(QVU):
            qvproj(QVU * j + t)
        return carry

    with _scope("ph_qv"):
        jax.lax.fori_loop(0, NX // QVU, qv_body, 0)

    row_q = jax.lax.broadcasted_iota(jnp.int32, (LANES, TQ), 0)
    QPC = TQ // R1
    s_bufs = ((sa_ref, sa2_ref), (sb_ref, sb2_ref))
    m_bufs = (ma_ref, mb_ref)

    def load_q(b):
        hd = b // NQ
        qt = b % NQ
        lo = hd * DH
        g = lo // LANES
        o = lo % LANES
        st = o > LANES - DH
        g = jnp.where(st, 5, g)
        o = jnp.where(st, (lo // LANES) * DH, o)
        q = jnp.concatenate([qt_ref[g, qt * QPC + t] for t in range(QPC)], axis=1).astype(f32)
        q = jnp.where((row_q >= o) & (row_q < o + DH), q, 0.0).astype(bf16)
        return q, g

    def qk_task(q, g, c, par, m8, z):
        s = jnp.dot(k_ref[g, c * TC:(c + 1) * TC, :], q, preferred_element_type=f32)
        s_ref = s_bufs[par][c // HALF]
        r = (c % HALF) * TC
        if z is None:
            s_ref[r:r + TC, :] = s
        else:
            s_ref[pl.ds(pl.multiple_of(r + z, 8), TC), :] = s
        cm = jnp.max(s.reshape(TC // 8, 8, TQ), axis=0)
        m8 = cm if m8 is None else jnp.maximum(m8, cm)
        if z is not None and MDL and c % MDL == MDL - 1:
            s_ref[pl.ds(pl.multiple_of(S // 2 + z, 8), 8), :] = m8
        return m8

    def pv_task(hd, c, par, m, acc):
        r = (c % HALF) * TC
        p = jnp.exp2(s_bufs[par][c // HALF][r:r + TC, :] - m).astype(bf16)
        k0 = c * TC
        v = vt_ref[hd, k0 // R1][:, k0 % R1:k0 % R1 + TC]
        o = jnp.dot(v, p, preferred_element_type=f32)
        return o if acc is None else acc + o

    modb_cp.wait()
    wg_cp.wait()
    wu_cp.wait()
    mod_ref[:, 2 * D:6 * D] = jnp.dot(sc, wmod_ref[:, 2 * D:6 * D], preferred_element_type=f32)
    wgul_ref[0:FREM, :] = wgt_ref[FMAIN:F, :]
    wgul_ref[FREM:2 * FREM, :] = wut_ref[FMAIN:F, :]

    q0, g0 = load_q(0)
    m8 = None
    for c in range(NC):
        m8 = qk_task(q0, g0, c, 0, m8, None)
    ma_ref[...] = jnp.max(m8, axis=0, keepdims=True)
    q0, g0 = load_q(1)
    m8 = None
    for c in range(SKEW):
        m8 = qk_task(q0, g0, c, 1, m8, None)
    m8_ref[...] = m8

    def attn_steps(j, last):
        b0 = NSTEP * j
        z = zero_ref[0]
        m8 = m8_ref[...]
        q = g = None
        acc = m = None
        for i in range(NSTEP * NC):
            tq, cq = divmod(i + NC + SKEW, NC)
            tp, cp_ = divmod(i, NC)
            if not (last and tq >= NSTEP):
                if q is None or cq == 0:
                    q, g = load_q(b0 + tq)
                m8 = qk_task(q, g, cq, tq % 2, None if cq == 0 else m8, z)
                if cq == NC - 1:
                    m_bufs[tq % 2][...] = jnp.max(m8, axis=0, keepdims=True)
            if cp_ == 0:
                m = m_bufs[tp % 2][...]
                acc = None
            hd = (b0 + tp) // NQ
            acc = pv_task(hd, cp_, tp % 2, m, acc)
            if cp_ == NC - 1:
                ot_ref[hd, (b0 + tp) % NQ] = acc * (1.0 / acc[DH:DH + 1, :])
        if not last:
            m8_ref[...] = m8

    def attn_body(j, carry):
        attn_steps(j, False)
        return carry

    with _scope("ph_attn"):
        jax.lax.fori_loop(0, NB // NSTEP - 1, attn_body, 0)
    with _scope("ph_attn_tail"):
        attn_steps(NB // NSTEP - 1, True)

    wo_cp.wait()
    wd_cp.wait()
    ga = mod_ref[0:1, 2 * D:3 * D]
    sb = mod_ref[0:1, 3 * D:4 * D]
    cb1 = 1.0 + mod_ref[0:1, 4 * D:5 * D]
    gb = mod_ref[0:1, 5 * D:6 * D]
    per3 = TQ // R3

    def rows(par):
        if isinstance(par, int):
            return pl.ds(par * R3, R3)
        return pl.ds(pl.multiple_of(par * R3, R3), R3)

    def stage_a1(i, par):
        qt = i // per3
        sub = i % per3
        for hd in range(H):
            full = ot_ref[hd, qt]
            blk = full[:, 0:R3]
            for t in range(1, per3):
                blk = jnp.where(sub == t, full[:, t * R3:(t + 1) * R3], blk)
            oc_ref[DH * hd:DH * hd + DH, :] = blk[0:DH]
        oo_ref[rows(par), :] = oc_ref[0:D, :].astype(bf16).T

    def stage_a2(i, par):
        r0 = pl.multiple_of(i * R3, R3)
        attn = jnp.dot(oo_ref[rows(par), :], wo_ref[...], preferred_element_type=f32)
        x1 = x_ref[pl.ds(r0, R3), :].astype(f32) + ga * attn
        x1_ref[rows(par), :] = x1
        hh_ref[rows(par), :] = (_layernorm(x1) * cb1 + sb).astype(bf16)

    def ffn_part(h2, f0, fc, y):
        g = jax.lax.dot_general(h2, wgt_ref[f0:f0 + fc, :], _NT, preferred_element_type=f32)
        u = jax.lax.dot_general(h2, wut_ref[f0:f0 + fc, :], _NT, preferred_element_type=f32)
        a = (jax.nn.gelu(g, approximate=True) * u).astype(bf16)
        d = jnp.dot(a, wd_ref[f0:f0 + fc, :], preferred_element_type=f32)
        return d if y is None else y + d

    def ffn_step(i, par, do_a2, do_a1):
        r0 = pl.multiple_of(i * R3, R3)
        h2 = hh_ref[rows(par), :]
        gu = jax.lax.dot_general(h2, wgul_ref[...], _NT, preferred_element_type=f32)
        a = (jax.nn.gelu(gu[:, 0:FREM], approximate=True) * gu[:, FREM:2 * FREM]).astype(bf16)
        y = jnp.dot(a, wd_ref[FMAIN:F, :], preferred_element_type=f32)
        f0 = 0
        for n, fc in enumerate(FCS):
            if n == LATEPOS and do_a2:
                h2 = hh_ref[rows(par), :]
            y = ffn_part(h2, f0, fc, y)
            f0 += fc
            if n + 1 == MIDPOS:
                if do_a2:
                    stage_a2(i + 1, 1 - par)
                if do_a1:
                    stage_a1(jnp.minimum(i + 2, N3 - 1), par)
        assert f0 == FMAIN
        ostage_ref[pl.ds(r0, R3), :] = (x1_ref[rows(par), :] + gb * y).astype(bf16)
        cp(ostage_ref.at[pl.ds(r0, R3), :], out_hbm.at[pl.ds(r0, R3), :], _S_OUT).start()

    stage_a1(0, 0)
    stage_a2(0, 0)
    stage_a1(1, 1)

    def ffn_body(i, carry):
        ffn_step(i, i % 2, True, True)
        return carry

    with _scope("ph_ffn"):
        jax.lax.fori_loop(0, N3 - 1, ffn_body, 0)
    with _scope("ph_ffn_tail"):
        ffn_step(N3 - 1, (N3 - 1) % 2, False, False)
    cp(ostage_ref, out_hbm, _S_OUT).wait()


@jax.jit
def pallas_adaLN_cond__mha_block__geglu_ffn__prompt_kernel(
    A_x: jax.Array,
    A_wqkv: jax.Array,
    A_wo: jax.Array,
    B_x: jax.Array,
    B_w_gate: jax.Array,
    B_w_up: jax.Array,
    B_w_down: jax.Array,
    c: jax.Array,
    w_mod: jax.Array,
):
    del B_x
    f32 = jnp.float32
    bf16 = jnp.bfloat16
    x2 = A_x.reshape(S, D)
    any_spec = pl.BlockSpec(memory_space=pl.ANY)
    out = pl.pallas_call(
        _kernel,
        out_shape=jax.ShapeDtypeStruct((S, D), A_x.dtype),
        in_specs=[any_spec] * 8,
        out_specs=any_spec,
        scratch_shapes=[
            pltpu.VMEM((S, D), bf16),
            pltpu.VMEM((D, 3 * D), bf16),
            pltpu.VMEM((D, D), bf16),
            pltpu.VMEM((F, D), bf16),
            pltpu.VMEM((F, D), bf16),
            pltpu.VMEM((F, D), bf16),
            pltpu.VMEM((1, D), bf16),
            pltpu.VMEM((D, 6 * D), bf16),
            pltpu.VMEM((S, D), bf16),
            pltpu.VMEM((16, 6 * D), f32),
            pltpu.VMEM((2 * D, D), bf16),
            pltpu.VMEM((NX, R1, D), bf16),
            pltpu.VMEM((LANES, R1), f32),
            pltpu.VMEM((D + 16, R1), f32),
            pltpu.VMEM((2 * FREM, D), bf16),
            pltpu.VMEM((NG, S, LANES), bf16),
            pltpu.VMEM((NG, NX, LANES, R1), bf16),
            pltpu.VMEM((H, NX, VR, R1), bf16),
            pltpu.VMEM((H, NQ, VR, TQ), f32),
            pltpu.VMEM((S // 2 + 8, TQ), f32),
            pltpu.VMEM((S // 2 + 8, TQ), f32),
            pltpu.VMEM((S // 2 + 8, TQ), f32),
            pltpu.VMEM((S // 2 + 8, TQ), f32),
            pltpu.VMEM((1, TQ), f32),
            pltpu.VMEM((1, TQ), f32),
            pltpu.VMEM((8, TQ), f32),
            pltpu.VMEM((D + 16, R1), f32),
            pltpu.VMEM((2 * R1, D), bf16),
            pltpu.VMEM((2 * R3, D), f32),
            pltpu.VMEM((2 * R3, D), bf16),
            pltpu.SMEM((1,), jnp.int32),
            pltpu.SemaphoreType.DMA((14,)),
        ],
        compiler_params=pltpu.CompilerParams(vmem_limit_bytes=110 * 1024 * 1024),
        name="adaln_block",
    )(x2, A_wqkv, A_wo, B_w_gate.T, B_w_up.T, B_w_down, c, w_mod)
    return out.reshape(A_x.shape)
```

```python
import math

import jax
import jax.numpy as jnp
import jax.experimental.pallas as pl
import jax.experimental.pallas.tpu as pltpu

S = 2048
D = 640
H = 32
DH = 20
F = 1728
LANES = 128
NG = 6
TQ = 512
NQ = S // TQ
TC = LANES
NC = S // TC
HALF = NC // 2
NB = H * NQ
NSTEP = 8
SKEW = 1
VR = 32
R1 = 256
NX = S // R1
R3 = 256
N3 = S // R3
FCS = (384, 640, 640)
MIDPOS = 1
LATEPOS = 2
EPS = 1e-5
QSCALE = (DH ** -0.5) * math.log2(math.e)
STRADDLE = [h for h in range(H) if (DH * h) % LANES > LANES - DH]
FMAIN = (F // LANES) * LANES
FREM = F - FMAIN
MDL = 2
KE = 4
XEARLY = 2

_NT = (((1,), (1,)), ((), ()))

(_S_C, _S_MODA, _S_MODA2, _S_WQ, _S_WK, _S_WV, _S_MODB, _S_WO, _S_WG, _S_WU, _S_WD, _S_OUT, _S_XA,
 _S_XB) = range(14)


def _layernorm(xf):
    m = jnp.mean(xf, axis=-1, keepdims=True)
    xc = xf - m
    v = jnp.mean(xc * xc, axis=-1, keepdims=True)
    return xc * jax.lax.rsqrt(v + EPS)


def _kernel(x_hbm, wqkv_hbm, wo_hbm, wgt_hbm, wut_hbm, wd_hbm, c_hbm, wmod_hbm,
            out_hbm,
            x_ref, wqkv_ref, wo_ref, wgt_ref, wut_ref, wd_ref, c_ref, wmod_ref, ostage_ref,
            mod_ref, wt_ref, h_ref, qx_ref, ov_ref, wgul_ref,
            k_ref, qt_ref, vt_ref, ot_ref,
            sa_ref, sa2_ref, sb_ref, sb2_ref, ma_ref, mb_ref, m8_ref, oc_ref,
            hh_ref, x1_ref, oo_ref,
            zero_ref, sems):
    f32 = jnp.float32
    bf16 = jnp.bfloat16

    def cp(src, dst, slot):
        return pltpu.make_async_copy(src, dst, sems.at[slot])

    XE = XEARLY * R1
    c_cp = cp(c_hbm, c_ref, _S_C)
    moda_cp = cp(wmod_hbm.at[:, 0:2 * D], wmod_ref.at[:, 0:2 * D], _S_MODA)
    modb_cp = cp(wmod_hbm.at[:, 2 * D:6 * D], wmod_ref.at[:, 2 * D:6 * D], _S_MODB)
    wq_cp = cp(wqkv_hbm.at[:, 0:D], wqkv_ref.at[:, 0:D], _S_WQ)
    wk_cp = cp(wqkv_hbm.at[:, D:2 * D], wqkv_ref.at[:, D:2 * D], _S_WK)
    wv_cp = cp(wqkv_hbm.at[:, 2 * D:3 * D], wqkv_ref.at[:, 2 * D:3 * D], _S_WV)
    wo_cp = cp(wo_hbm, wo_ref, _S_WO)
    wg_cp = cp(wgt_hbm, wgt_ref, _S_WG)
    wu_cp = cp(wut_hbm, wut_ref, _S_WU)
    wd_cp = cp(wd_hbm, wd_ref, _S_WD)
    xa_cp = cp(x_hbm.at[0:XE, :], x_ref.at[0:XE, :], _S_XA)
    XM = 2 * XE
    xb_cp = cp(x_hbm.at[XE:XM, :], x_ref.at[XE:XM, :], _S_XB)
    xc_cp = cp(x_hbm.at[XM:S, :], x_ref.at[XM:S, :], _S_MODA2)

    zero_ref[0] = 0
    c_cp.start()
    xa_cp.start()
    moda_cp.start()
    wk_cp.start()

    c_cp.wait()
    c = c_ref[...].astype(f32)
    sc = jnp.broadcast_to((c * jax.nn.sigmoid(c)).astype(bf16), (16, D))
    xa_cp.wait()
    xn0 = _layernorm(x_ref[0:R1, :].astype(f32))
    moda_cp.wait()
    xb_cp.start()
    wq_cp.start()
    wv_cp.start()
    xc_cp.start()
    mod_ref[:, 0:2 * D] = jnp.dot(sc, wmod_ref[:, 0:2 * D], preferred_element_type=f32)
    sa = mod_ref[0:1, 0 * D:1 * D]
    ca1 = 1.0 + mod_ref[0:1, 1 * D:2 * D]

    def chunk_rows(i):
        if isinstance(i, int):
            return pl.ds(i * R1, R1)
        return pl.ds(pl.multiple_of(i * R1, R1), R1)

    def ln1(i):
        xf = x_ref[chunk_rows(i), :].astype(f32)
        h_ref[i] = (_layernorm(xf) * ca1 + sa).astype(bf16)

    lane_k = jax.lax.broadcasted_iota(jnp.int32, (R1, LANES), 1)

    def kproj(i):
        h = h_ref[i]
        kk = jnp.dot(h, wqkv_ref[:, D:2 * D], preferred_element_type=f32)
        for g in range(5):
            k_ref[g, chunk_rows(i), :] = kk[:, g * LANES:(g + 1) * LANES].astype(bf16)
        kx = jnp.zeros((R1, LANES), f32)
        for j, hd in enumerate(STRADDLE):
            lo = DH * hd
            t = lo // LANES
            sh = (DH * j - lo) % LANES
            a = pltpu.roll(kk[:, t * LANES:(t + 1) * LANES], sh, 1)
            b = pltpu.roll(kk[:, (t + 1) * LANES:(t + 2) * LANES], sh, 1)
            n_a = (t + 1) * LANES - lo
            kx = jnp.where((lane_k >= DH * j) & (lane_k < DH * j + n_a), a,
                           jnp.where((lane_k >= DH * j + n_a) & (lane_k < DH * (j + 1)), b, kx))
        k_ref[5, chunk_rows(i), :] = kx.astype(bf16)

    row32 = jax.lax.broadcasted_iota(jnp.int32, (VR, R1), 0)

    def qvproj(i):
        h = h_ref[i]
        qv = jax.lax.dot_general(wt_ref[...], h, _NT, preferred_element_type=f32)
        oc_ref[0:D, :] = qv[0:D] * QSCALE
        for g in range(5):
            qt_ref[g, i] = oc_ref[g * LANES:(g + 1) * LANES, :].astype(bf16)
        for j, hd in enumerate(STRADDLE):
            qx_ref[DH * j:DH * (j + 1), :] = oc_ref[DH * hd:DH * (hd + 1), :]
        qt_ref[5, i] = qx_ref[...].astype(bf16)
        ov_ref[0:D, :] = qv[D:2 * D]
        for hd in range(H):
            a0 = (DH * hd // 8) * 8
            off = DH * hd - a0
            win = ov_ref[a0:a0 + VR + 8, :]
            win = win[off:off + VR]
            win = jnp.where(row32 < DH, win, jnp.where(row32 == DH, 1.0, 0.0))
            vt_ref[hd, i] = win.astype(bf16)

    qx_ref[...] = jnp.zeros(qx_ref.shape, f32)
    ov_ref[D:D + 16, :] = jnp.zeros((16, R1), f32)
    h_ref[0] = (xn0 * ca1 + sa).astype(bf16)
    wk_cp.wait()
    for i in range(KE):
        if i + 1 == XEARLY:
            xb_cp.wait()
        if i + 1 == 2 * XEARLY or (i == KE - 1 and KE < 2 * XEARLY):
            xc_cp.wait()
            modb_cp.start()
            wo_cp.start()
            wg_cp.start()
            wu_cp.start()
            wd_cp.start()
        if i == KE - 1:
            wq_cp.wait()
            wv_cp.wait()
            wt_ref[0:D, :] = wqkv_ref[:, 0:D].T
            wt_ref[D:2 * D, :] = wqkv_ref[:, 2 * D:3 * D].T
        ln1(i + 1)
        kproj(i)

    def full_body(i, carry):
        qvproj(i)
        ln1(jnp.minimum(i + 1, NX - 1))
        kproj(i)
        return carry

    jax.lax.fori_loop(KE, NX, full_body, 0)

    def qv_body(i, carry):
        qvproj(i)
        return carry

    jax.lax.fori_loop(0, KE, qv_body, 0)

    row_q = jax.lax.broadcasted_iota(jnp.int32, (LANES, TQ), 0)
    QPC = TQ // R1
    per3 = TQ // R3
    s_bufs = ((sa_ref, sa2_ref), (sb_ref, sb2_ref))
    m_bufs = (ma_ref, mb_ref)

    def load_q(b):
        hd = b // NQ
        qt = b % NQ
        lo = hd * DH
        g = lo // LANES
        o = lo % LANES
        st = o > LANES - DH
        g = jnp.where(st, 5, g)
        o = jnp.where(st, (lo // LANES) * DH, o)
        q = jnp.concatenate([qt_ref[g, qt * QPC + t] for t in range(QPC)], axis=1).astype(f32)
        q = jnp.where((row_q >= o) & (row_q < o + DH), q, 0.0).astype(bf16)
        return q, g

    def qk_task(q, g, c, par, m8, z):
        s = jnp.dot(k_ref[g, c * TC:(c + 1) * TC, :], q, preferred_element_type=f32)
        s_ref = s_bufs[par][c // HALF]
        r = (c % HALF) * TC
        if z is None:
            s_ref[r:r + TC, :] = s
        else:
            s_ref[pl.ds(pl.multiple_of(r + z, 8), TC), :] = s
        cm = jnp.max(s.reshape(TC // 8, 8, TQ), axis=0)
        m8 = cm if m8 is None else jnp.maximum(m8, cm)
        if z is not None and MDL and c % MDL == MDL - 1:
            s_ref[pl.ds(pl.multiple_of(S // 2 + z, 8), 8), :] = m8
        return m8

    def pv_task(hd, c, par, m, acc):
        r = (c % HALF) * TC
        p = jnp.exp2(s_bufs[par][c // HALF][r:r + TC, :] - m).astype(bf16)
        k0 = c * TC
        v = vt_ref[hd, k0 // R1][:, k0 % R1:k0 % R1 + TC]
        o = jnp.dot(v, p, preferred_element_type=f32)
        return o if acc is None else acc + o

    modb_cp.wait()
    wg_cp.wait()
    wu_cp.wait()
    wo_cp.wait()
    wd_cp.wait()
    mod_ref[:, 2 * D:6 * D] = jnp.dot(sc, wmod_ref[:, 2 * D:6 * D], preferred_element_type=f32)
    wgul_ref[0:FREM, :] = wgt_ref[FMAIN:F, :]
    wgul_ref[FREM:2 * FREM, :] = wut_ref[FMAIN:F, :]

    q0, g0 = load_q(0)
    m8 = None
    for c in range(NC):
        m8 = qk_task(q0, g0, c, 0, m8, None)
    ma_ref[...] = jnp.max(m8, axis=0, keepdims=True)
    q0, g0 = load_q(1)
    m8 = None
    for c in range(SKEW):
        m8 = qk_task(q0, g0, c, 1, m8, None)
    m8_ref[...] = m8

    def attn_steps(j, last):
        b0 = NSTEP * j
        z = zero_ref[0]
        m8 = m8_ref[...]
        q = g = None
        acc = m = None
        for i in range(NSTEP * NC):
            tq, cq = divmod(i + NC + SKEW, NC)
            tp, cp_ = divmod(i, NC)
            if not (last and tq >= NSTEP):
                if q is None or cq == 0:
                    q, g = load_q(b0 + tq)
                m8 = qk_task(q, g, cq, tq % 2, None if cq == 0 else m8, z)
                if cq == NC - 1:
                    m_bufs[tq % 2][...] = jnp.max(m8, axis=0, keepdims=True)
            if cp_ == 0:
                m = m_bufs[tp % 2][...]
                acc = None
            hd = (b0 + tp) // NQ
            acc = pv_task(hd, cp_, tp % 2, m, acc)
            if cp_ == NC - 1:
                o = acc * (1.0 / acc[DH:DH + 1, :])
                for t in range(per3):
                    ot_ref[hd, ((b0 + tp) % NQ) * per3 + t] = o[:, t * R3:(t + 1) * R3]
        if not last:
            m8_ref[...] = m8

    def attn_body(j, carry):
        attn_steps(j, False)
        return carry

    jax.lax.fori_loop(0, NB // NSTEP - 1, attn_body, 0)
    attn_steps(NB // NSTEP - 1, True)

    ga = mod_ref[0:1, 2 * D:3 * D]
    sb = mod_ref[0:1, 3 * D:4 * D]
    cb1 = 1.0 + mod_ref[0:1, 4 * D:5 * D]
    gb = mod_ref[0:1, 5 * D:6 * D]
    def rows(par):
        if isinstance(par, int):
            return pl.ds(par * R3, R3)
        return pl.ds(pl.multiple_of(par * R3, R3), R3)

    def stage_a1(i, par):
        for hd in range(H):
            oc_ref[DH * hd:DH * hd + DH, :] = ot_ref[hd, i, 0:DH, :]
        oo_ref[rows(par), :] = oc_ref[0:D, :].astype(bf16).T

    def stage_a2(i, par):
        r0 = pl.multiple_of(i * R3, R3)
        attn = jnp.dot(oo_ref[rows(par), :], wo_ref[...], preferred_element_type=f32)
        x1 = x_ref[pl.ds(r0, R3), :].astype(f32) + ga * attn
        x1_ref[rows(par), :] = x1
        hh_ref[rows(par), :] = (_layernorm(x1) * cb1 + sb).astype(bf16)

    def ffn_part(h2, f0, fc, y):
        g = jax.lax.dot_general(h2, wgt_ref[f0:f0 + fc, :], _NT, preferred_element_type=f32)
        u = jax.lax.dot_general(h2, wut_ref[f0:f0 + fc, :], _NT, preferred_element_type=f32)
        a = (jax.nn.gelu(g, approximate=True) * u).astype(bf16)
        d = jnp.dot(a, wd_ref[f0:f0 + fc, :], preferred_element_type=f32)
        return d if y is None else y + d

    def ffn_step(i, par, do_a2, do_a1):
        r0 = pl.multiple_of(i * R3, R3)
        h2 = hh_ref[rows(par), :]
        gu = jax.lax.dot_general(h2, wgul_ref[...], _NT, preferred_element_type=f32)
        a = (jax.nn.gelu(gu[:, 0:FREM], approximate=True) * gu[:, FREM:2 * FREM]).astype(bf16)
        y = jnp.dot(a, wd_ref[FMAIN:F, :], preferred_element_type=f32)
        f0 = 0
        for n, fc in enumerate(FCS):
            if n == LATEPOS and do_a2:
                h2 = hh_ref[rows(par), :]
            y = ffn_part(h2, f0, fc, y)
            f0 += fc
            if n + 1 == MIDPOS:
                if do_a2:
                    stage_a2(i + 1, 1 - par)
                if do_a1:
                    stage_a1(jnp.minimum(i + 2, N3 - 1), par)
        assert f0 == FMAIN
        ostage_ref[pl.ds(r0, R3), :] = (x1_ref[rows(par), :] + gb * y).astype(bf16)
        cp(ostage_ref.at[pl.ds(r0, R3), :], out_hbm.at[pl.ds(r0, R3), :], _S_OUT).start()

    stage_a1(0, 0)
    stage_a2(0, 0)
    stage_a1(1, 1)

    def ffn_body(i, carry):
        ffn_step(i, i % 2, True, True)
        return carry

    jax.lax.fori_loop(0, N3 - 1, ffn_body, 0)
    ffn_step(N3 - 1, (N3 - 1) % 2, False, False)
    cp(ostage_ref, out_hbm, _S_OUT).wait()


@jax.jit
def pallas_adaLN_cond__mha_block__geglu_ffn__prompt_kernel(
    A_x: jax.Array,
    A_wqkv: jax.Array,
    A_wo: jax.Array,
    B_x: jax.Array,
    B_w_gate: jax.Array,
    B_w_up: jax.Array,
    B_w_down: jax.Array,
    c: jax.Array,
    w_mod: jax.Array,
):
    del B_x
    f32 = jnp.float32
    bf16 = jnp.bfloat16
    x2 = A_x.reshape(S, D)
    any_spec = pl.BlockSpec(memory_space=pl.ANY)
    out = pl.pallas_call(
        _kernel,
        out_shape=jax.ShapeDtypeStruct((S, D), A_x.dtype),
        in_specs=[any_spec] * 8,
        out_specs=any_spec,
        scratch_shapes=[
            pltpu.VMEM((S, D), bf16),
            pltpu.VMEM((D, 3 * D), bf16),
            pltpu.VMEM((D, D), bf16),
            pltpu.VMEM((F, D), bf16),
            pltpu.VMEM((F, D), bf16),
            pltpu.VMEM((F, D), bf16),
            pltpu.VMEM((1, D), bf16),
            pltpu.VMEM((D, 6 * D), bf16),
            pltpu.VMEM((S, D), bf16),
            pltpu.VMEM((16, 6 * D), f32),
            pltpu.VMEM((2 * D, D), bf16),
            pltpu.VMEM((NX, R1, D), bf16),
            pltpu.VMEM((LANES, R1), f32),
            pltpu.VMEM((D + 16, R1), f32),
            pltpu.VMEM((2 * FREM, D), bf16),
            pltpu.VMEM((NG, S, LANES), bf16),
            pltpu.VMEM((NG, NX, LANES, R1), bf16),
            pltpu.VMEM((H, NX, VR, R1), bf16),
            pltpu.VMEM((H, N3, VR, R3), f32),
            pltpu.VMEM((S // 2 + 8, TQ), f32),
            pltpu.VMEM((S // 2 + 8, TQ), f32),
            pltpu.VMEM((S // 2 + 8, TQ), f32),
            pltpu.VMEM((S // 2 + 8, TQ), f32),
            pltpu.VMEM((1, TQ), f32),
            pltpu.VMEM((1, TQ), f32),
            pltpu.VMEM((8, TQ), f32),
            pltpu.VMEM((D, R1), f32),
            pltpu.VMEM((2 * R1, D), bf16),
            pltpu.VMEM((2 * R3, D), f32),
            pltpu.VMEM((2 * R3, D), bf16),
            pltpu.SMEM((1,), jnp.int32),
            pltpu.SemaphoreType.DMA((14,)),
        ],
        compiler_params=pltpu.CompilerParams(vmem_limit_bytes=110 * 1024 * 1024),
        name="adaln_block",
    )(x2, A_wqkv, A_wo, B_w_gate.T, B_w_up.T, B_w_down, c, w_mod)
    return out.reshape(A_x.shape)
```

```python
import math

import jax
import jax.numpy as jnp
import jax.experimental.pallas as pl
import jax.experimental.pallas.tpu as pltpu

S = 2048
D = 640
H = 32
DH = 20
F = 1728
LANES = 128
NG = 6
TQ = 512
NQ = S // TQ
TC = LANES
NC = S // TC
HALF = NC // 2
NB = H * NQ
NSTEP = 8
SKEW = 1
VR = 32
R1 = 256
NX = S // R1
R3 = 256
N3 = S // R3
FCS = (384, 640, 640)
MIDPOS = 1
LATEPOS = 2
EPS = 1e-5
QSCALE = (DH ** -0.5) * math.log2(math.e)
STRADDLE = [h for h in range(H) if (DH * h) % LANES > LANES - DH]
FMAIN = (F // LANES) * LANES
FREM = F - FMAIN
MDL = 2
KE = 4
XEARLY = 2

_NT = (((1,), (1,)), ((), ()))

(_S_C, _S_MODA, _S_MODA2, _S_WQ, _S_WK, _S_WV, _S_MODB, _S_WO, _S_WG, _S_WU, _S_WD, _S_OUT, _S_XA,
 _S_XB) = range(14)


def _layernorm(xf):
    m = jnp.mean(xf, axis=-1, keepdims=True)
    xc = xf - m
    v = jnp.mean(xc * xc, axis=-1, keepdims=True)
    return xc * jax.lax.rsqrt(v + EPS)


def _kernel(x_hbm, wqkv_hbm, wo_hbm, wgt_hbm, wut_hbm, wd_hbm, c_hbm, wmod_hbm,
            out_hbm,
            x_ref, wqkv_ref, wo_ref, wgt_ref, wut_ref, wd_ref, c_ref, wmod_ref, ostage_ref,
            mod_ref, wt_ref, h_ref, oq_ref, qx_ref, ov_ref, wgul_ref,
            k_ref, qt_ref, vt_ref, ot_ref,
            sa_ref, sa2_ref, sb_ref, sb2_ref, ma_ref, mb_ref, m8_ref, oc_ref,
            hh_ref, x1_ref, oo_ref,
            zero_ref, sems):
    f32 = jnp.float32
    bf16 = jnp.bfloat16

    def cp(src, dst, slot):
        return pltpu.make_async_copy(src, dst, sems.at[slot])

    XE = XEARLY * R1
    c_cp = cp(c_hbm, c_ref, _S_C)
    moda_cp = cp(wmod_hbm.at[:, 0:2 * D], wmod_ref.at[:, 0:2 * D], _S_MODA)
    modb_cp = cp(wmod_hbm.at[:, 2 * D:6 * D], wmod_ref.at[:, 2 * D:6 * D], _S_MODB)
    wq_cp = cp(wqkv_hbm.at[:, 0:D], wqkv_ref.at[:, 0:D], _S_WQ)
    wk_cp = cp(wqkv_hbm.at[:, D:2 * D], wqkv_ref.at[:, D:2 * D], _S_WK)
    wv_cp = cp(wqkv_hbm.at[:, 2 * D:3 * D], wqkv_ref.at[:, 2 * D:3 * D], _S_WV)
    wo_cp = cp(wo_hbm, wo_ref, _S_WO)
    wg_cp = cp(wgt_hbm, wgt_ref, _S_WG)
    wu_cp = cp(wut_hbm, wut_ref, _S_WU)
    wd_cp = cp(wd_hbm, wd_ref, _S_WD)
    xa_cp = cp(x_hbm.at[0:XE, :], x_ref.at[0:XE, :], _S_XA)
    XM = 2 * XE
    xb_cp = cp(x_hbm.at[XE:XM, :], x_ref.at[XE:XM, :], _S_XB)
    xc_cp = cp(x_hbm.at[XM:S, :], x_ref.at[XM:S, :], _S_MODA2)

    zero_ref[0] = 0
    c_cp.start()
    xa_cp.start()
    moda_cp.start()
    wk_cp.start()

    c_cp.wait()
    c = c_ref[...].astype(f32)
    sc = jnp.broadcast_to((c * jax.nn.sigmoid(c)).astype(bf16), (16, D))
    xa_cp.wait()
    xn0 = _layernorm(x_ref[0:R1, :].astype(f32))
    moda_cp.wait()
    xb_cp.start()
    wq_cp.start()
    wv_cp.start()
    xc_cp.start()
    mod_ref[:, 0:2 * D] = jnp.dot(sc, wmod_ref[:, 0:2 * D], preferred_element_type=f32)
    sa = mod_ref[0:1, 0 * D:1 * D]
    ca1 = 1.0 + mod_ref[0:1, 1 * D:2 * D]

    def chunk_rows(i):
        if isinstance(i, int):
            return pl.ds(i * R1, R1)
        return pl.ds(pl.multiple_of(i * R1, R1), R1)

    def ln1(i):
        xf = x_ref[chunk_rows(i), :].astype(f32)
        h_ref[i] = (_layernorm(xf) * ca1 + sa).astype(bf16)

    lane_k = jax.lax.broadcasted_iota(jnp.int32, (R1, LANES), 1)

    def kproj(i):
        h = h_ref[i]
        kk = jnp.dot(h, wqkv_ref[:, D:2 * D], preferred_element_type=f32)
        for g in range(5):
            k_ref[g, chunk_rows(i), :] = kk[:, g * LANES:(g + 1) * LANES].astype(bf16)
        kx = jnp.zeros((R1, LANES), f32)
        for j, hd in enumerate(STRADDLE):
            lo = DH * hd
            t = lo // LANES
            sh = (DH * j - lo) % LANES
            a = pltpu.roll(kk[:, t * LANES:(t + 1) * LANES], sh, 1)
            b = pltpu.roll(kk[:, (t + 1) * LANES:(t + 2) * LANES], sh, 1)
            n_a = (t + 1) * LANES - lo
            kx = jnp.where((lane_k >= DH * j) & (lane_k < DH * j + n_a), a,
                           jnp.where((lane_k >= DH * j + n_a) & (lane_k < DH * (j + 1)), b, kx))
        k_ref[5, chunk_rows(i), :] = kx.astype(bf16)

    row32 = jax.lax.broadcasted_iota(jnp.int32, (VR, R1), 0)

    def qvproj(i):
        par = i % 2
        h = h_ref[i]
        qv = jax.lax.dot_general(wt_ref[...], h, _NT, preferred_element_type=f32)
        oq_ref[par] = qv[0:D] * QSCALE
        for g in range(5):
            qt_ref[g, i] = oq_ref[par, g * LANES:(g + 1) * LANES, :].astype(bf16)
        for j, hd in enumerate(STRADDLE):
            qx_ref[par, DH * j:DH * (j + 1), :] = oq_ref[par, DH * hd:DH * (hd + 1), :]
        qt_ref[5, i] = qx_ref[par].astype(bf16)
        ov_ref[par, 0:D, :] = qv[D:2 * D]
        for hd in range(H):
            a0 = (DH * hd // 8) * 8
            off = DH * hd - a0
            win = ov_ref[par, a0:a0 + VR + 8, :]
            win = win[off:off + VR]
            win = jnp.where(row32 < DH, win, jnp.where(row32 == DH, 1.0, 0.0))
            vt_ref[hd, i] = win.astype(bf16)

    qx_ref[...] = jnp.zeros(qx_ref.shape, f32)
    ov_ref[:, D:D + 16, :] = jnp.zeros((2, 16, R1), f32)
    h_ref[0] = (xn0 * ca1 + sa).astype(bf16)
    wk_cp.wait()
    for i in range(KE):
        if i + 1 == XEARLY:
            xb_cp.wait()
        if i + 1 == 2 * XEARLY or (i == KE - 1 and KE < 2 * XEARLY):
            xc_cp.wait()
            modb_cp.start()
            wo_cp.start()
            wg_cp.start()
            wu_cp.start()
            wd_cp.start()
        if i == KE - 1:
            wq_cp.wait()
            wv_cp.wait()
            wt_ref[0:D, :] = wqkv_ref[:, 0:D].T
            wt_ref[D:2 * D, :] = wqkv_ref[:, 2 * D:3 * D].T
        ln1(i + 1)
        kproj(i)

    for i in range(KE, NX):
        qvproj(i)
        if i + 1 < NX:
            ln1(i + 1)
        kproj(i)
    for i in range(KE):
        qvproj(i)

    row_q = jax.lax.broadcasted_iota(jnp.int32, (LANES, TQ), 0)
    QPC = TQ // R1
    per3 = TQ // R3
    s_bufs = ((sa_ref, sa2_ref), (sb_ref, sb2_ref))
    m_bufs = (ma_ref, mb_ref)

    def load_q(b):
        hd = b // NQ
        qt = b % NQ
        lo = hd * DH
        g = lo // LANES
        o = lo % LANES
        st = o > LANES - DH
        g = jnp.where(st, 5, g)
        o = jnp.where(st, (lo // LANES) * DH, o)
        q = jnp.concatenate([qt_ref[g, qt * QPC + t] for t in range(QPC)], axis=1).astype(f32)
        q = jnp.where((row_q >= o) & (row_q < o + DH), q, 0.0).astype(bf16)
        return q, g

    def qk_task(q, g, c, par, m8, z):
        s = jnp.dot(k_ref[g, c * TC:(c + 1) * TC, :], q, preferred_element_type=f32)
        s_ref = s_bufs[par][c // HALF]
        r = (c % HALF) * TC
        if z is None:
            s_ref[r:r + TC, :] = s
        else:
            s_ref[pl.ds(pl.multiple_of(r + z, 8), TC), :] = s
        cm = jnp.max(s.reshape(TC // 8, 8, TQ), axis=0)
        m8 = cm if m8 is None else jnp.maximum(m8, cm)
        if z is not None and MDL and c % MDL == MDL - 1:
            s_ref[pl.ds(pl.multiple_of(S // 2 + z, 8), 8), :] = m8
        return m8

    def pv_task(hd, c, par, m, acc):
        r = (c % HALF) * TC
        p = jnp.exp2(s_bufs[par][c // HALF][r:r + TC, :] - m).astype(bf16)
        k0 = c * TC
        v = vt_ref[hd, k0 // R1][:, k0 % R1:k0 % R1 + TC]
        o = jnp.dot(v, p, preferred_element_type=f32)
        return o if acc is None else acc + o

    modb_cp.wait()
    wg_cp.wait()
    wu_cp.wait()
    wo_cp.wait()
    wd_cp.wait()
    mod_ref[:, 2 * D:6 * D] = jnp.dot(sc, wmod_ref[:, 2 * D:6 * D], preferred_element_type=f32)
    wgul_ref[0:FREM, :] = wgt_ref[FMAIN:F, :]
    wgul_ref[FREM:2 * FREM, :] = wut_ref[FMAIN:F, :]

    q0, g0 = load_q(0)
    m8 = None
    for c in range(NC):
        m8 = qk_task(q0, g0, c, 0, m8, None)
    ma_ref[...] = jnp.max(m8, axis=0, keepdims=True)
    q0, g0 = load_q(1)
    m8 = None
    for c in range(SKEW):
        m8 = qk_task(q0, g0, c, 1, m8, None)
    m8_ref[...] = m8

    def attn_steps(j, last):
        b0 = NSTEP * j
        z = zero_ref[0]
        m8 = m8_ref[...]
        q = g = None
        acc = m = None
        for i in range(NSTEP * NC):
            tq, cq = divmod(i + NC + SKEW, NC)
            tp, cp_ = divmod(i, NC)
            if not (last and tq >= NSTEP):
                if q is None or cq == 0:
                    q, g = load_q(b0 + tq)
                m8 = qk_task(q, g, cq, tq % 2, None if cq == 0 else m8, z)
                if cq == NC - 1:
                    m_bufs[tq % 2][...] = jnp.max(m8, axis=0, keepdims=True)
            if cp_ == 0:
                m = m_bufs[tp % 2][...]
                acc = None
            hd = (b0 + tp) // NQ
            acc = pv_task(hd, cp_, tp % 2, m, acc)
            if cp_ == NC - 1:
                o = acc * (1.0 / acc[DH:DH + 1, :])
                for t in range(per3):
                    ot_ref[hd, ((b0 + tp) % NQ) * per3 + t] = o[:, t * R3:(t + 1) * R3]
        if not last:
            m8_ref[...] = m8

    def attn_body(j, carry):
        attn_steps(j, False)
        return carry

    jax.lax.fori_loop(0, NB // NSTEP - 1, attn_body, 0)
    attn_steps(NB // NSTEP - 1, True)

    ga = mod_ref[0:1, 2 * D:3 * D]
    sb = mod_ref[0:1, 3 * D:4 * D]
    cb1 = 1.0 + mod_ref[0:1, 4 * D:5 * D]
    gb = mod_ref[0:1, 5 * D:6 * D]
    def rows(par):
        if isinstance(par, int):
            return pl.ds(par * R3, R3)
        return pl.ds(pl.multiple_of(par * R3, R3), R3)

    def stage_a1(i, par):
        for hd in range(H):
            oc_ref[DH * hd:DH * hd + DH, :] = ot_ref[hd, i, 0:DH, :]
        oo_ref[rows(par), :] = oc_ref[0:D, :].astype(bf16).T

    def stage_a2(i, par):
        r0 = i * R3
        attn = jnp.dot(oo_ref[rows(par), :], wo_ref[...], preferred_element_type=f32)
        x1 = x_ref[pl.ds(r0, R3), :].astype(f32) + ga * attn
        x1_ref[rows(par), :] = x1
        hh_ref[rows(par), :] = (_layernorm(x1) * cb1 + sb).astype(bf16)

    def ffn_part(h2, f0, fc, y):
        g = jax.lax.dot_general(h2, wgt_ref[f0:f0 + fc, :], _NT, preferred_element_type=f32)
        u = jax.lax.dot_general(h2, wut_ref[f0:f0 + fc, :], _NT, preferred_element_type=f32)
        a = (jax.nn.gelu(g, approximate=True) * u).astype(bf16)
        d = jnp.dot(a, wd_ref[f0:f0 + fc, :], preferred_element_type=f32)
        return d if y is None else y + d

    def ffn_step(i, par, do_a2, do_a1):
        r0 = i * R3
        h2 = hh_ref[rows(par), :]
        gu = jax.lax.dot_general(h2, wgul_ref[...], _NT, preferred_element_type=f32)
        a = (jax.nn.gelu(gu[:, 0:FREM], approximate=True) * gu[:, FREM:2 * FREM]).astype(bf16)
        y = jnp.dot(a, wd_ref[FMAIN:F, :], preferred_element_type=f32)
        f0 = 0
        for n, fc in enumerate(FCS):
            if n == LATEPOS and do_a2:
                h2 = hh_ref[rows(par + zero_ref[0]), :]
            y = ffn_part(h2, f0, fc, y)
            f0 += fc
            if n + 1 == MIDPOS:
                if do_a2:
                    stage_a2(i + 1, 1 - par)
                if do_a1:
                    stage_a1(i + 2, par)
        assert f0 == FMAIN
        ostage_ref[pl.ds(r0, R3), :] = (x1_ref[rows(par), :] + gb * y).astype(bf16)
        cp(ostage_ref.at[pl.ds(r0, R3), :], out_hbm.at[pl.ds(r0, R3), :], _S_OUT).start()

    stage_a1(0, 0)
    stage_a2(0, 0)
    stage_a1(1, 1)

    for i in range(N3):
        ffn_step(i, i % 2, i + 1 < N3, i + 2 < N3)
    cp(ostage_ref, out_hbm, _S_OUT).wait()


@jax.jit
def pallas_adaLN_cond__mha_block__geglu_ffn__prompt_kernel(
    A_x: jax.Array,
    A_wqkv: jax.Array,
    A_wo: jax.Array,
    B_x: jax.Array,
    B_w_gate: jax.Array,
    B_w_up: jax.Array,
    B_w_down: jax.Array,
    c: jax.Array,
    w_mod: jax.Array,
):
    del B_x
    f32 = jnp.float32
    bf16 = jnp.bfloat16
    x2 = A_x.reshape(S, D)
    any_spec = pl.BlockSpec(memory_space=pl.ANY)
    out = pl.pallas_call(
        _kernel,
        out_shape=jax.ShapeDtypeStruct((S, D), A_x.dtype),
        in_specs=[any_spec] * 8,
        out_specs=any_spec,
        scratch_shapes=[
            pltpu.VMEM((S, D), bf16),
            pltpu.VMEM((D, 3 * D), bf16),
            pltpu.VMEM((D, D), bf16),
            pltpu.VMEM((F, D), bf16),
            pltpu.VMEM((F, D), bf16),
            pltpu.VMEM((F, D), bf16),
            pltpu.VMEM((1, D), bf16),
            pltpu.VMEM((D, 6 * D), bf16),
            pltpu.VMEM((S, D), bf16),
            pltpu.VMEM((16, 6 * D), f32),
            pltpu.VMEM((2 * D, D), bf16),
            pltpu.VMEM((NX, R1, D), bf16),
            pltpu.VMEM((2, D, R1), f32),
            pltpu.VMEM((2, LANES, R1), f32),
            pltpu.VMEM((2, D + 16, R1), f32),
            pltpu.VMEM((2 * FREM, D), bf16),
            pltpu.VMEM((NG, S, LANES), bf16),
            pltpu.VMEM((NG, NX, LANES, R1), bf16),
            pltpu.VMEM((H, NX, VR, R1), bf16),
            pltpu.VMEM((H, N3, VR, R3), f32),
            pltpu.VMEM((S // 2 + 8, TQ), f32),
            pltpu.VMEM((S // 2 + 8, TQ), f32),
            pltpu.VMEM((S // 2 + 8, TQ), f32),
            pltpu.VMEM((S // 2 + 8, TQ), f32),
            pltpu.VMEM((1, TQ), f32),
            pltpu.VMEM((1, TQ), f32),
            pltpu.VMEM((8, TQ), f32),
            pltpu.VMEM((D, R1), f32),
            pltpu.VMEM((2 * R1, D), bf16),
            pltpu.VMEM((2 * R3, D), f32),
            pltpu.VMEM((2 * R3, D), bf16),
            pltpu.SMEM((1,), jnp.int32),
            pltpu.SemaphoreType.DMA((14,)),
        ],
        compiler_params=pltpu.CompilerParams(vmem_limit_bytes=110 * 1024 * 1024),
        name="adaln_block",
    )(x2, A_wqkv, A_wo, B_w_gate.T, B_w_up.T, B_w_down, c, w_mod)
    return out.reshape(A_x.shape)
```

```python
import math

import jax
import jax.numpy as jnp
import jax.experimental.pallas as pl
import jax.experimental.pallas.tpu as pltpu

S = 2048
D = 640
H = 32
DH = 20
F = 1728
LANES = 128
NG = 6
TQ = 512
NQ = S // TQ
TC = LANES
NC = S // TC
HALF = NC // 2
NB = H * NQ
NSTEP = 8
SKEW = 1
VR = 32
R1 = 256
NX = S // R1
R3 = 256
N3 = S // R3
FCS = (384, 640, 640)
MIDPOS = 1
LATEPOS = 2
EPS = 1e-5
QSCALE = (DH ** -0.5) * math.log2(math.e)
STRADDLE = [h for h in range(H) if (DH * h) % LANES > LANES - DH]
FMAIN = (F // LANES) * LANES
FREM = F - FMAIN
MDL = 2
KE = 4
XEARLY = 2

_NT = (((1,), (1,)), ((), ()))

(_S_C, _S_MODA, _S_MODB, _S_WQ, _S_WK, _S_WV, _S_WO, _S_WG, _S_WU, _S_WD, _S_XA, _S_XB, _S_XC,
 _S_OUT) = range(14)


def _layernorm(xf):
    m = jnp.mean(xf, axis=-1, keepdims=True)
    xc = xf - m
    v = jnp.mean(xc * xc, axis=-1, keepdims=True)
    return xc * jax.lax.rsqrt(v + EPS)


def _kernel(x_hbm, wqkv_hbm, wo_hbm, wgt_hbm, wut_hbm, wd_hbm, c_hbm, wmod_hbm,
            out_hbm,
            x_ref, wqkv_ref, wo_ref, wgt_ref, wut_ref, wd_ref, c_ref, wmod_ref, ostage_ref,
            mod_ref, wt_ref, h_ref, oq_ref, qx_ref, ov_ref, wgul_ref,
            k_ref, qt_ref, vt_ref, ot_ref,
            sa_ref, sa2_ref, sb_ref, sb2_ref, ma_ref, mb_ref, m8_ref, oc_ref,
            hh_ref, x1_ref, oo_ref,
            zero_ref, sems):
    f32 = jnp.float32
    bf16 = jnp.bfloat16

    def cp(src, dst, slot):
        return pltpu.make_async_copy(src, dst, sems.at[slot])

    XE = XEARLY * R1
    c_cp = cp(c_hbm, c_ref, _S_C)
    moda_cp = cp(wmod_hbm.at[:, 0:2 * D], wmod_ref.at[:, 0:2 * D], _S_MODA)
    modb_cp = cp(wmod_hbm.at[:, 2 * D:6 * D], wmod_ref.at[:, 2 * D:6 * D], _S_MODB)
    wq_cp = cp(wqkv_hbm.at[:, 0:D], wqkv_ref.at[:, 0:D], _S_WQ)
    wk_cp = cp(wqkv_hbm.at[:, D:2 * D], wqkv_ref.at[:, D:2 * D], _S_WK)
    wv_cp = cp(wqkv_hbm.at[:, 2 * D:3 * D], wqkv_ref.at[:, 2 * D:3 * D], _S_WV)
    wo_cp = cp(wo_hbm, wo_ref, _S_WO)
    wg_cp = cp(wgt_hbm, wgt_ref, _S_WG)
    wu_cp = cp(wut_hbm, wut_ref, _S_WU)
    wd_cp = cp(wd_hbm, wd_ref, _S_WD)
    xa_cp = cp(x_hbm.at[0:XE, :], x_ref.at[0:XE, :], _S_XA)
    XM = 2 * XE
    xb_cp = cp(x_hbm.at[XE:XM, :], x_ref.at[XE:XM, :], _S_XB)
    xc_cp = cp(x_hbm.at[XM:S, :], x_ref.at[XM:S, :], _S_XC)

    zero_ref[0] = 0
    c_cp.start()
    xa_cp.start()
    moda_cp.start()
    wk_cp.start()

    c_cp.wait()
    c = c_ref[...].astype(f32)
    sc = jnp.broadcast_to((c * jax.nn.sigmoid(c)).astype(bf16), (16, D))
    xa_cp.wait()
    xn0 = _layernorm(x_ref[0:R1, :].astype(f32))
    moda_cp.wait()
    xb_cp.start()
    wq_cp.start()
    wv_cp.start()
    xc_cp.start()
    mod_ref[:, 0:2 * D] = jnp.dot(sc, wmod_ref[:, 0:2 * D], preferred_element_type=f32)
    sa = mod_ref[0:1, 0 * D:1 * D]
    ca1 = 1.0 + mod_ref[0:1, 1 * D:2 * D]

    def chunk_rows(i):
        if isinstance(i, int):
            return pl.ds(i * R1, R1)
        return pl.ds(pl.multiple_of(i * R1, R1), R1)

    def ln1(i):
        xf = x_ref[chunk_rows(i), :].astype(f32)
        h_ref[i] = (_layernorm(xf) * ca1 + sa).astype(bf16)

    lane_k = jax.lax.broadcasted_iota(jnp.int32, (R1, LANES), 1)

    def kproj(i):
        h = h_ref[i]
        kk = jnp.dot(h, wqkv_ref[:, D:2 * D], preferred_element_type=f32)
        for g in range(5):
            k_ref[g, chunk_rows(i), :] = kk[:, g * LANES:(g + 1) * LANES].astype(bf16)
        kx = jnp.zeros((R1, LANES), f32)
        for j, hd in enumerate(STRADDLE):
            lo = DH * hd
            t = lo // LANES
            sh = (DH * j - lo) % LANES
            a = pltpu.roll(kk[:, t * LANES:(t + 1) * LANES], sh, 1)
            b = pltpu.roll(kk[:, (t + 1) * LANES:(t + 2) * LANES], sh, 1)
            n_a = (t + 1) * LANES - lo
            kx = jnp.where((lane_k >= DH * j) & (lane_k < DH * j + n_a), a,
                           jnp.where((lane_k >= DH * j + n_a) & (lane_k < DH * (j + 1)), b, kx))
        k_ref[5, chunk_rows(i), :] = kx.astype(bf16)

    row32 = jax.lax.broadcasted_iota(jnp.int32, (VR, R1), 0)

    def qvproj(i):
        par = i % 2
        h = h_ref[i]
        qv = jax.lax.dot_general(wt_ref[...], h, _NT, preferred_element_type=f32)
        oq_ref[par] = qv[0:D] * QSCALE
        for g in range(5):
            qt_ref[g, i] = oq_ref[par, g * LANES:(g + 1) * LANES, :].astype(bf16)
        for j, hd in enumerate(STRADDLE):
            qx_ref[par, DH * j:DH * (j + 1), :] = oq_ref[par, DH * hd:DH * (hd + 1), :]
        qt_ref[5, i] = qx_ref[par].astype(bf16)
        ov_ref[par, 0:D, :] = qv[D:2 * D]
        for hd in range(H):
            a0 = (DH * hd // 8) * 8
            off = DH * hd - a0
            win = ov_ref[par, a0:a0 + VR + 8, :]
            win = win[off:off + VR]
            win = jnp.where(row32 < DH, win, jnp.where(row32 == DH, 1.0, 0.0))
            vt_ref[hd, i] = win.astype(bf16)

    qx_ref[...] = jnp.zeros(qx_ref.shape, f32)
    ov_ref[:, D:D + 16, :] = jnp.zeros((2, 16, R1), f32)
    h_ref[0] = (xn0 * ca1 + sa).astype(bf16)
    wk_cp.wait()
    for i in range(KE):
        if i + 1 == XEARLY:
            xb_cp.wait()
        if i + 1 == 2 * XEARLY:
            xc_cp.wait()
            modb_cp.start()
            wo_cp.start()
            wg_cp.start()
            wu_cp.start()
            wd_cp.start()
        if i == KE - 1:
            wq_cp.wait()
            wv_cp.wait()
            wt_ref[0:D, :] = wqkv_ref[:, 0:D].T
            wt_ref[D:2 * D, :] = wqkv_ref[:, 2 * D:3 * D].T
        ln1(i + 1)
        kproj(i)

    for i in range(KE, NX):
        qvproj(i)
        if i + 1 < NX:
            ln1(i + 1)
        kproj(i)
    for i in range(KE):
        qvproj(i)

    row_q = jax.lax.broadcasted_iota(jnp.int32, (LANES, TQ), 0)
    QPC = TQ // R1
    per3 = TQ // R3
    s_bufs = ((sa_ref, sa2_ref), (sb_ref, sb2_ref))
    m_bufs = (ma_ref, mb_ref)

    def load_q(b):
        hd = b // NQ
        qt = b % NQ
        lo = hd * DH
        g = lo // LANES
        o = lo % LANES
        st = o > LANES - DH
        g = jnp.where(st, 5, g)
        o = jnp.where(st, (lo // LANES) * DH, o)
        q = jnp.concatenate([qt_ref[g, qt * QPC + t] for t in range(QPC)], axis=1).astype(f32)
        q = jnp.where((row_q >= o) & (row_q < o + DH), q, 0.0).astype(bf16)
        return q, g

    def qk_task(q, g, c, par, m8, z):
        s = jnp.dot(k_ref[g, c * TC:(c + 1) * TC, :], q, preferred_element_type=f32)
        s_ref = s_bufs[par][c // HALF]
        r = (c % HALF) * TC
        if z is None:
            s_ref[r:r + TC, :] = s
        else:
            s_ref[pl.ds(pl.multiple_of(r + z, 8), TC), :] = s
        cm = jnp.max(s.reshape(TC // 8, 8, TQ), axis=0)
        m8 = cm if m8 is None else jnp.maximum(m8, cm)
        if z is not None and c % MDL == MDL - 1:
            s_ref[pl.ds(pl.multiple_of(S // 2 + z, 8), 8), :] = m8
        return m8

    def pv_task(hd, c, par, m, acc):
        r = (c % HALF) * TC
        p = jnp.exp2(s_bufs[par][c // HALF][r:r + TC, :] - m).astype(bf16)
        k0 = c * TC
        v = vt_ref[hd, k0 // R1][:, k0 % R1:k0 % R1 + TC]
        o = jnp.dot(v, p, preferred_element_type=f32)
        return o if acc is None else acc + o

    modb_cp.wait()
    wg_cp.wait()
    wu_cp.wait()
    wo_cp.wait()
    wd_cp.wait()
    mod_ref[:, 2 * D:6 * D] = jnp.dot(sc, wmod_ref[:, 2 * D:6 * D], preferred_element_type=f32)
    wgul_ref[0:FREM, :] = wgt_ref[FMAIN:F, :]
    wgul_ref[FREM:2 * FREM, :] = wut_ref[FMAIN:F, :]

    q0, g0 = load_q(0)
    m8 = None
    for c in range(NC):
        m8 = qk_task(q0, g0, c, 0, m8, None)
    ma_ref[...] = jnp.max(m8, axis=0, keepdims=True)
    q0, g0 = load_q(1)
    m8 = None
    for c in range(SKEW):
        m8 = qk_task(q0, g0, c, 1, m8, None)
    m8_ref[...] = m8

    def attn_steps(j, last):
        b0 = NSTEP * j
        z = zero_ref[0]
        m8 = m8_ref[...]
        q = g = None
        acc = m = None
        for i in range(NSTEP * NC):
            tq, cq = divmod(i + NC + SKEW, NC)
            tp, cp_ = divmod(i, NC)
            if not (last and tq >= NSTEP):
                if q is None or cq == 0:
                    q, g = load_q(b0 + tq)
                m8 = qk_task(q, g, cq, tq % 2, None if cq == 0 else m8, z)
                if cq == NC - 1:
                    m_bufs[tq % 2][...] = jnp.max(m8, axis=0, keepdims=True)
            if cp_ == 0:
                m = m_bufs[tp % 2][...]
                acc = None
            hd = (b0 + tp) // NQ
            acc = pv_task(hd, cp_, tp % 2, m, acc)
            if cp_ == NC - 1:
                o = acc * (1.0 / acc[DH:DH + 1, :])
                for t in range(per3):
                    ot_ref[hd, ((b0 + tp) % NQ) * per3 + t] = o[:, t * R3:(t + 1) * R3]
        if not last:
            m8_ref[...] = m8

    def attn_body(j, carry):
        attn_steps(j, False)
        return carry

    jax.lax.fori_loop(0, NB // NSTEP - 1, attn_body, 0)
    attn_steps(NB // NSTEP - 1, True)

    ga = mod_ref[0:1, 2 * D:3 * D]
    sb = mod_ref[0:1, 3 * D:4 * D]
    cb1 = 1.0 + mod_ref[0:1, 4 * D:5 * D]
    gb = mod_ref[0:1, 5 * D:6 * D]

    def rows(par):
        if isinstance(par, int):
            return pl.ds(par * R3, R3)
        return pl.ds(pl.multiple_of(par * R3, R3), R3)

    def stage_a1(i, par):
        for hd in range(H):
            oc_ref[DH * hd:DH * hd + DH, :] = ot_ref[hd, i, 0:DH, :]
        oo_ref[rows(par), :] = oc_ref[0:D, :].astype(bf16).T

    def stage_a2(i, par):
        r0 = i * R3
        attn = jnp.dot(oo_ref[rows(par), :], wo_ref[...], preferred_element_type=f32)
        x1 = x_ref[pl.ds(r0, R3), :].astype(f32) + ga * attn
        x1_ref[rows(par), :] = x1
        hh_ref[rows(par), :] = (_layernorm(x1) * cb1 + sb).astype(bf16)

    def ffn_part(h2, f0, fc, y):
        g = jax.lax.dot_general(h2, wgt_ref[f0:f0 + fc, :], _NT, preferred_element_type=f32)
        u = jax.lax.dot_general(h2, wut_ref[f0:f0 + fc, :], _NT, preferred_element_type=f32)
        a = (jax.nn.gelu(g, approximate=True) * u).astype(bf16)
        d = jnp.dot(a, wd_ref[f0:f0 + fc, :], preferred_element_type=f32)
        return d if y is None else y + d

    def ffn_step(i, par, do_a2, do_a1):
        r0 = i * R3
        h2 = hh_ref[rows(par), :]
        gu = jax.lax.dot_general(h2, wgul_ref[...], _NT, preferred_element_type=f32)
        a = (jax.nn.gelu(gu[:, 0:FREM], approximate=True) * gu[:, FREM:2 * FREM]).astype(bf16)
        y = jnp.dot(a, wd_ref[FMAIN:F, :], preferred_element_type=f32)
        f0 = 0
        for n, fc in enumerate(FCS):
            if n == LATEPOS and do_a2:
                h2 = hh_ref[rows(par + zero_ref[0]), :]
            y = ffn_part(h2, f0, fc, y)
            f0 += fc
            if n + 1 == MIDPOS:
                if do_a2:
                    stage_a2(i + 1, 1 - par)
                if do_a1:
                    stage_a1(i + 2, par)
        assert f0 == FMAIN
        ostage_ref[pl.ds(r0, R3), :] = (x1_ref[rows(par), :] + gb * y).astype(bf16)
        cp(ostage_ref.at[pl.ds(r0, R3), :], out_hbm.at[pl.ds(r0, R3), :], _S_OUT).start()

    stage_a1(0, 0)
    stage_a2(0, 0)
    stage_a1(1, 1)

    for i in range(N3):
        ffn_step(i, i % 2, i + 1 < N3, i + 2 < N3)
    cp(ostage_ref, out_hbm, _S_OUT).wait()


@jax.jit
def pallas_adaLN_cond__mha_block__geglu_ffn__prompt_kernel(
    A_x: jax.Array,
    A_wqkv: jax.Array,
    A_wo: jax.Array,
    B_x: jax.Array,
    B_w_gate: jax.Array,
    B_w_up: jax.Array,
    B_w_down: jax.Array,
    c: jax.Array,
    w_mod: jax.Array,
):
    del B_x
    f32 = jnp.float32
    bf16 = jnp.bfloat16
    x2 = A_x.reshape(S, D)
    any_spec = pl.BlockSpec(memory_space=pl.ANY)
    out = pl.pallas_call(
        _kernel,
        out_shape=jax.ShapeDtypeStruct((S, D), A_x.dtype),
        in_specs=[any_spec] * 8,
        out_specs=any_spec,
        scratch_shapes=[
            pltpu.VMEM((S, D), bf16),
            pltpu.VMEM((D, 3 * D), bf16),
            pltpu.VMEM((D, D), bf16),
            pltpu.VMEM((F, D), bf16),
            pltpu.VMEM((F, D), bf16),
            pltpu.VMEM((F, D), bf16),
            pltpu.VMEM((1, D), bf16),
            pltpu.VMEM((D, 6 * D), bf16),
            pltpu.VMEM((S, D), bf16),
            pltpu.VMEM((16, 6 * D), f32),
            pltpu.VMEM((2 * D, D), bf16),
            pltpu.VMEM((NX, R1, D), bf16),
            pltpu.VMEM((2, D, R1), f32),
            pltpu.VMEM((2, LANES, R1), f32),
            pltpu.VMEM((2, D + 16, R1), f32),
            pltpu.VMEM((2 * FREM, D), bf16),
            pltpu.VMEM((NG, S, LANES), bf16),
            pltpu.VMEM((NG, NX, LANES, R1), bf16),
            pltpu.VMEM((H, NX, VR, R1), bf16),
            pltpu.VMEM((H, N3, VR, R3), f32),
            pltpu.VMEM((S // 2 + 8, TQ), f32),
            pltpu.VMEM((S // 2 + 8, TQ), f32),
            pltpu.VMEM((S // 2 + 8, TQ), f32),
            pltpu.VMEM((S // 2 + 8, TQ), f32),
            pltpu.VMEM((1, TQ), f32),
            pltpu.VMEM((1, TQ), f32),
            pltpu.VMEM((8, TQ), f32),
            pltpu.VMEM((D, R1), f32),
            pltpu.VMEM((2 * R1, D), bf16),
            pltpu.VMEM((2 * R3, D), f32),
            pltpu.VMEM((2 * R3, D), bf16),
            pltpu.SMEM((1,), jnp.int32),
            pltpu.SemaphoreType.DMA((14,)),
        ],
        compiler_params=pltpu.CompilerParams(vmem_limit_bytes=110 * 1024 * 1024),
        name="adaln_block",
    )(x2, A_wqkv, A_wo, B_w_gate.T, B_w_up.T, B_w_down, c, w_mod)
    return out.reshape(A_x.shape)
```

```python
import math

import jax
import jax.numpy as jnp
import jax.experimental.pallas as pl
import jax.experimental.pallas.tpu as pltpu

S = 2048
D = 640
H = 32
DH = 20
F = 1728
LANES = 128
NG = 6
TQ = 512
NQ = S // TQ
TC = LANES
NC = S // TC
HALF = NC // 2
NB = H * NQ
NSTEP = 8
SKEW = 1
VR = 32
R1 = 256
NX = S // R1
R3 = 256
N3 = S // R3
FCS = (384, 640, 640)
MIDPOS = 1
LATEPOS = 2
EPS = 1e-5
QSCALE = (DH ** -0.5) * math.log2(math.e)
STRADDLE = [h for h in range(H) if (DH * h) % LANES > LANES - DH]
FMAIN = (F // LANES) * LANES
FREM = F - FMAIN
MDL = 2
KE = 4
XEARLY = 2

_NT = (((1,), (1,)), ((), ()))

(_S_C, _S_MODA, _S_MODB, _S_WQ, _S_WK, _S_WV, _S_WO, _S_WG, _S_WU, _S_WD, _S_XA, _S_XB, _S_XC,
 _S_OUT) = range(14)


def _layernorm(xf):
    m = jnp.mean(xf, axis=-1, keepdims=True)
    xc = xf - m
    v = jnp.mean(xc * xc, axis=-1, keepdims=True)
    return xc * jax.lax.rsqrt(v + EPS)


def _kernel(x_hbm, wqkv_hbm, wo_hbm, wgt_hbm, wut_hbm, wd_hbm, c_hbm, wmod_hbm,
            out_hbm,
            x_ref, wqkv_ref, wo_ref, wgt_ref, wut_ref, wd_ref, c_ref, wmod_ref, ostage_ref,
            mod_ref, wt_ref, h_ref, oq_ref, qx_ref, ov_ref, wgul_ref,
            k_ref, qt_ref, vt_ref, ot_ref,
            sa_ref, sa2_ref, sb_ref, sb2_ref, ma_ref, mb_ref, m8_ref, oc_ref,
            hh_ref, x1_ref, oo_ref,
            zero_ref, sems):
    f32 = jnp.float32
    bf16 = jnp.bfloat16

    def cp(src, dst, slot):
        return pltpu.make_async_copy(src, dst, sems.at[slot])

    XE = XEARLY * R1
    c_cp = cp(c_hbm, c_ref, _S_C)
    moda_cp = cp(wmod_hbm.at[:, 0:2 * D], wmod_ref.at[:, 0:2 * D], _S_MODA)
    modb_cp = cp(wmod_hbm.at[:, 2 * D:6 * D], wmod_ref.at[:, 2 * D:6 * D], _S_MODB)
    wq_cp = cp(wqkv_hbm.at[:, 0:D], wqkv_ref.at[:, 0:D], _S_WQ)
    wk_cp = cp(wqkv_hbm.at[:, D:2 * D], wqkv_ref.at[:, D:2 * D], _S_WK)
    wv_cp = cp(wqkv_hbm.at[:, 2 * D:3 * D], wqkv_ref.at[:, 2 * D:3 * D], _S_WV)
    wo_cp = cp(wo_hbm, wo_ref, _S_WO)
    wg_cp = cp(wgt_hbm, wgt_ref, _S_WG)
    wu_cp = cp(wut_hbm, wut_ref, _S_WU)
    wd_cp = cp(wd_hbm, wd_ref, _S_WD)
    xa_cp = cp(x_hbm.at[0:XE, :], x_ref.at[0:XE, :], _S_XA)
    XM = 2 * XE
    xb_cp = cp(x_hbm.at[XE:XM, :], x_ref.at[XE:XM, :], _S_XB)
    xc_cp = cp(x_hbm.at[XM:S, :], x_ref.at[XM:S, :], _S_XC)

    zero_ref[0] = 0
    c_cp.start()
    xa_cp.start()
    moda_cp.start()
    wk_cp.start()

    c_cp.wait()
    c = c_ref[...].astype(f32)
    sc = jnp.broadcast_to((c * jax.nn.sigmoid(c)).astype(bf16), (16, D))
    xa_cp.wait()
    xn0 = _layernorm(x_ref[0:R1, :].astype(f32))
    moda_cp.wait()
    xb_cp.start()
    wq_cp.start()
    wv_cp.start()
    xc_cp.start()
    mod_ref[:, 0:2 * D] = jnp.dot(sc, wmod_ref[:, 0:2 * D], preferred_element_type=f32)
    sa = mod_ref[0:1, 0 * D:1 * D]
    ca1 = 1.0 + mod_ref[0:1, 1 * D:2 * D]

    def chunk_rows(i):
        if isinstance(i, int):
            return pl.ds(i * R1, R1)
        return pl.ds(pl.multiple_of(i * R1, R1), R1)

    def ln1(i):
        xf = x_ref[chunk_rows(i), :].astype(f32)
        h_ref[i] = (_layernorm(xf) * ca1 + sa).astype(bf16)

    lane_k = jax.lax.broadcasted_iota(jnp.int32, (R1, LANES), 1)

    def kproj(i):
        h = h_ref[i]
        kk = jnp.dot(h, wqkv_ref[:, D:2 * D], preferred_element_type=f32)
        for g in range(5):
            k_ref[g, chunk_rows(i), :] = kk[:, g * LANES:(g + 1) * LANES].astype(bf16)
        kx = jnp.zeros((R1, LANES), f32)
        for j, hd in enumerate(STRADDLE):
            lo = DH * hd
            t = lo // LANES
            sh = (DH * j - lo) % LANES
            a = pltpu.roll(kk[:, t * LANES:(t + 1) * LANES], sh, 1)
            b = pltpu.roll(kk[:, (t + 1) * LANES:(t + 2) * LANES], sh, 1)
            n_a = (t + 1) * LANES - lo
            kx = jnp.where((lane_k >= DH * j) & (lane_k < DH * j + n_a), a,
                           jnp.where((lane_k >= DH * j + n_a) & (lane_k < DH * (j + 1)), b, kx))
        k_ref[5, chunk_rows(i), :] = kx.astype(bf16)

    row32 = jax.lax.broadcasted_iota(jnp.int32, (VR, R1), 0)

    def qvproj(i):
        par = i % 2
        h = h_ref[i]
        qv = jax.lax.dot_general(wt_ref[...], h, _NT, preferred_element_type=f32)
        oq_ref[par] = qv[0:D] * QSCALE
        for g in range(5):
            qt_ref[g, i] = oq_ref[par, g * LANES:(g + 1) * LANES, :].astype(bf16)
        for j, hd in enumerate(STRADDLE):
            qx_ref[par, DH * j:DH * (j + 1), :] = oq_ref[par, DH * hd:DH * (hd + 1), :]
        qt_ref[5, i] = qx_ref[par].astype(bf16)
        ov_ref[par, 0:D, :] = qv[D:2 * D]
        for hd in range(H):
            a0 = (DH * hd // 8) * 8
            off = DH * hd - a0
            win = ov_ref[par, a0:a0 + VR + 8, :]
            win = win[off:off + VR]
            win = jnp.where(row32 < DH, win, jnp.where(row32 == DH, 1.0, 0.0))
            vt_ref[hd, i] = win.astype(bf16)

    qx_ref[...] = jnp.zeros(qx_ref.shape, f32)
    ov_ref[:, D:D + 16, :] = jnp.zeros((2, 16, R1), f32)
    h_ref[0] = (xn0 * ca1 + sa).astype(bf16)
    wk_cp.wait()
    for i in range(KE):
        if i + 1 == XEARLY:
            xb_cp.wait()
        if i + 1 == 2 * XEARLY:
            xc_cp.wait()
        if i == KE - 1:
            wq_cp.wait()
            wv_cp.wait()
            wt_ref[0:D, :] = wqkv_ref[:, 0:D].T
            wt_ref[D:2 * D, :] = wqkv_ref[:, 2 * D:3 * D].T
        ln1(i + 1)
        kproj(i)

    for i in range(KE, NX):
        qvproj(i)
        if i + 1 < NX:
            ln1(i + 1)
        kproj(i)
    for i in range(KE):
        qvproj(i)

    row_q = jax.lax.broadcasted_iota(jnp.int32, (LANES, TQ), 0)
    QPC = TQ // R1
    per3 = TQ // R3
    s_bufs = ((sa_ref, sa2_ref), (sb_ref, sb2_ref))
    m_bufs = (ma_ref, mb_ref)

    def load_q(b):
        hd = b // NQ
        qt = b % NQ
        lo = hd * DH
        g = lo // LANES
        o = lo % LANES
        st = o > LANES - DH
        g = jnp.where(st, 5, g)
        o = jnp.where(st, (lo // LANES) * DH, o)
        q = jnp.concatenate([qt_ref[g, qt * QPC + t] for t in range(QPC)], axis=1).astype(f32)
        q = jnp.where((row_q >= o) & (row_q < o + DH), q, 0.0).astype(bf16)
        return q, g

    def qk_task(q, g, c, par, m8, z):
        s = jnp.dot(k_ref[g, c * TC:(c + 1) * TC, :], q, preferred_element_type=f32)
        s_ref = s_bufs[par][c // HALF]
        r = (c % HALF) * TC
        if z is None:
            s_ref[r:r + TC, :] = s
        else:
            s_ref[pl.ds(pl.multiple_of(r + z, 8), TC), :] = s
        cm = jnp.max(s.reshape(TC // 8, 8, TQ), axis=0)
        m8 = cm if m8 is None else jnp.maximum(m8, cm)
        if z is not None and c % MDL == MDL - 1:
            s_ref[pl.ds(pl.multiple_of(S // 2 + z, 8), 8), :] = m8
        return m8

    def pv_task(hd, c, par, m, acc):
        r = (c % HALF) * TC
        p = jnp.exp2(s_bufs[par][c // HALF][r:r + TC, :] - m).astype(bf16)
        k0 = c * TC
        v = vt_ref[hd, k0 // R1][:, k0 % R1:k0 % R1 + TC]
        o = jnp.dot(v, p, preferred_element_type=f32)
        return o if acc is None else acc + o

    modb_cp.start()
    wo_cp.start()
    wg_cp.start()
    wu_cp.start()
    wd_cp.start()

    q0, g0 = load_q(0)
    m8 = None
    for c in range(NC):
        m8 = qk_task(q0, g0, c, 0, m8, None)
    ma_ref[...] = jnp.max(m8, axis=0, keepdims=True)
    q0, g0 = load_q(1)
    m8 = None
    for c in range(SKEW):
        m8 = qk_task(q0, g0, c, 1, m8, None)
    m8_ref[...] = m8

    def attn_steps(j, last):
        b0 = NSTEP * j
        z = zero_ref[0]
        m8 = m8_ref[...]
        q = g = None
        acc = m = None
        for i in range(NSTEP * NC):
            tq, cq = divmod(i + NC + SKEW, NC)
            tp, cp_ = divmod(i, NC)
            if not (last and tq >= NSTEP):
                if q is None or cq == 0:
                    q, g = load_q(b0 + tq)
                m8 = qk_task(q, g, cq, tq % 2, None if cq == 0 else m8, z)
                if cq == NC - 1:
                    m_bufs[tq % 2][...] = jnp.max(m8, axis=0, keepdims=True)
            if cp_ == 0:
                m = m_bufs[tp % 2][...]
                acc = None
            hd = (b0 + tp) // NQ
            acc = pv_task(hd, cp_, tp % 2, m, acc)
            if cp_ == NC - 1:
                o = acc * (1.0 / acc[DH:DH + 1, :])
                for t in range(per3):
                    ot_ref[hd, ((b0 + tp) % NQ) * per3 + t] = o[:, t * R3:(t + 1) * R3]
        if not last:
            m8_ref[...] = m8

    def attn_body(j, carry):
        attn_steps(j, False)
        return carry

    jax.lax.fori_loop(0, NB // NSTEP - 1, attn_body, 0)
    modb_cp.wait()
    wg_cp.wait()
    wu_cp.wait()
    wo_cp.wait()
    wd_cp.wait()
    mod_ref[:, 2 * D:6 * D] = jnp.dot(sc, wmod_ref[:, 2 * D:6 * D], preferred_element_type=f32)
    wgul_ref[0:FREM, :] = wgt_ref[FMAIN:F, :]
    wgul_ref[FREM:2 * FREM, :] = wut_ref[FMAIN:F, :]

    attn_steps(NB // NSTEP - 1, True)

    ga = mod_ref[0:1, 2 * D:3 * D]
    sb = mod_ref[0:1, 3 * D:4 * D]
    cb1 = 1.0 + mod_ref[0:1, 4 * D:5 * D]
    gb = mod_ref[0:1, 5 * D:6 * D]

    def rows(par):
        if isinstance(par, int):
            return pl.ds(par * R3, R3)
        return pl.ds(pl.multiple_of(par * R3, R3), R3)

    def stage_a1(i, par):
        for hd in range(H):
            oc_ref[DH * hd:DH * hd + DH, :] = ot_ref[hd, i, 0:DH, :]
        oo_ref[rows(par), :] = oc_ref[0:D, :].astype(bf16).T

    def stage_a2(i, par):
        r0 = i * R3
        attn = jnp.dot(oo_ref[rows(par), :], wo_ref[...], preferred_element_type=f32)
        x1 = x_ref[pl.ds(r0, R3), :].astype(f32) + ga * attn
        x1_ref[rows(par), :] = x1
        hh_ref[rows(par), :] = (_layernorm(x1) * cb1 + sb).astype(bf16)

    def ffn_part(h2, f0, fc, y):
        g = jax.lax.dot_general(h2, wgt_ref[f0:f0 + fc, :], _NT, preferred_element_type=f32)
        u = jax.lax.dot_general(h2, wut_ref[f0:f0 + fc, :], _NT, preferred_element_type=f32)
        a = (jax.nn.gelu(g, approximate=True) * u).astype(bf16)
        d = jnp.dot(a, wd_ref[f0:f0 + fc, :], preferred_element_type=f32)
        return d if y is None else y + d

    def ffn_step(i, par, do_a2, do_a1):
        r0 = i * R3
        h2 = hh_ref[rows(par), :]
        gu = jax.lax.dot_general(h2, wgul_ref[...], _NT, preferred_element_type=f32)
        a = (jax.nn.gelu(gu[:, 0:FREM], approximate=True) * gu[:, FREM:2 * FREM]).astype(bf16)
        y = jnp.dot(a, wd_ref[FMAIN:F, :], preferred_element_type=f32)
        f0 = 0
        for n, fc in enumerate(FCS):
            if n == LATEPOS and do_a2:
                h2 = hh_ref[rows(par + zero_ref[0]), :]
            y = ffn_part(h2, f0, fc, y)
            f0 += fc
            if n + 1 == MIDPOS:
                if do_a2:
                    stage_a2(i + 1, 1 - par)
                if do_a1:
                    stage_a1(i + 2, par)
        assert f0 == FMAIN
        ostage_ref[pl.ds(r0, R3), :] = (x1_ref[rows(par), :] + gb * y).astype(bf16)
        cp(ostage_ref.at[pl.ds(r0, R3), :], out_hbm.at[pl.ds(r0, R3), :], _S_OUT).start()

    stage_a1(0, 0)
    stage_a2(0, 0)
    stage_a1(1, 1)

    for i in range(N3):
        ffn_step(i, i % 2, i + 1 < N3, i + 2 < N3)
    cp(ostage_ref, out_hbm, _S_OUT).wait()


@jax.jit
def pallas_adaLN_cond__mha_block__geglu_ffn__prompt_kernel(
    A_x: jax.Array,
    A_wqkv: jax.Array,
    A_wo: jax.Array,
    B_x: jax.Array,
    B_w_gate: jax.Array,
    B_w_up: jax.Array,
    B_w_down: jax.Array,
    c: jax.Array,
    w_mod: jax.Array,
):
    del B_x
    f32 = jnp.float32
    bf16 = jnp.bfloat16
    x2 = A_x.reshape(S, D)
    any_spec = pl.BlockSpec(memory_space=pl.ANY)
    out = pl.pallas_call(
        _kernel,
        out_shape=jax.ShapeDtypeStruct((S, D), A_x.dtype),
        in_specs=[any_spec] * 8,
        out_specs=any_spec,
        scratch_shapes=[
            pltpu.VMEM((S, D), bf16),
            pltpu.VMEM((D, 3 * D), bf16),
            pltpu.VMEM((D, D), bf16),
            pltpu.VMEM((F, D), bf16),
            pltpu.VMEM((F, D), bf16),
            pltpu.VMEM((F, D), bf16),
            pltpu.VMEM((1, D), bf16),
            pltpu.VMEM((D, 6 * D), bf16),
            pltpu.VMEM((S, D), bf16),
            pltpu.VMEM((16, 6 * D), f32),
            pltpu.VMEM((2 * D, D), bf16),
            pltpu.VMEM((NX, R1, D), bf16),
            pltpu.VMEM((2, D, R1), f32),
            pltpu.VMEM((2, LANES, R1), f32),
            pltpu.VMEM((2, D + 16, R1), f32),
            pltpu.VMEM((2 * FREM, D), bf16),
            pltpu.VMEM((NG, S, LANES), bf16),
            pltpu.VMEM((NG, NX, LANES, R1), bf16),
            pltpu.VMEM((H, NX, VR, R1), bf16),
            pltpu.VMEM((H, N3, VR, R3), f32),
            pltpu.VMEM((S // 2 + 8, TQ), f32),
            pltpu.VMEM((S // 2 + 8, TQ), f32),
            pltpu.VMEM((S // 2 + 8, TQ), f32),
            pltpu.VMEM((S // 2 + 8, TQ), f32),
            pltpu.VMEM((1, TQ), f32),
            pltpu.VMEM((1, TQ), f32),
            pltpu.VMEM((8, TQ), f32),
            pltpu.VMEM((D, R1), f32),
            pltpu.VMEM((2 * R1, D), bf16),
            pltpu.VMEM((2 * R3, D), f32),
            pltpu.VMEM((2 * R3, D), bf16),
            pltpu.SMEM((1,), jnp.int32),
            pltpu.SemaphoreType.DMA((14,)),
        ],
        compiler_params=pltpu.CompilerParams(vmem_limit_bytes=110 * 1024 * 1024),
        name="adaln_block",
    )(x2, A_wqkv, A_wo, B_w_gate.T, B_w_up.T, B_w_down, c, w_mod)
    return out.reshape(A_x.shape)
```
